```python
import jax
import jax.numpy as jnp

def _softmax(x, axis=-1):
    return jax.nn.softmax(x, axis=axis)
def _gelu(x):
    return jax.nn.gelu(x, approximate=True)
def _silu(x):
    return jax.nn.silu(x)
def _sigmoid(x):
    return jax.nn.sigmoid(x)
def _layernorm(x, axis=-1, eps=1e-5):
    m = jnp.mean(x, axis=axis, keepdims=True)
    v = jnp.var(x, axis=axis, keepdims=True)
    return (x - m) / jnp.sqrt(v + eps)
def _scatter_add(tgt, idx, src, axis=0):
    return tgt.at[idx].add(src)
def _segment_sum(src, seg, n):
    return jax.ops.segment_sum(src, seg, n)
class _Rng:
    def __init__(self, key):
        self._k = key
    def _next(self):
        self._k, sub = jax.random.split(self._k)
        return sub
    def normal(self, shape):
        return jax.random.normal(self._next(), shape, dtype=jnp.bfloat16)
    def randint(self, lo, hi, shape):
        return jax.random.randint(self._next(), shape, lo, hi, dtype=jnp.int32)
    def uniform(self, shape, lo=0.0, hi=1.0):
        return jax.random.uniform(self._next(), shape, jnp.bfloat16, lo, hi)
    def permutation(self, n):
        return jax.random.permutation(self._next(), n)


kernel_name = 'parallel_sum__sliding_local_dilated__glu_gated_geglu__prompt'

def setup_inputs():
    _rng = _Rng(jax.random.key(int.from_bytes(__import__("os").urandom(4), "little")))
    _w = (lambda a: (lambda t: t.astype(jnp.bfloat16) if jnp.issubdtype(t.dtype, jnp.floating) else t)(jnp.asarray(a)))
    def _A_setup():
        B, S, D = 1, 2048, 1024
        return {
            "x": _w((lambda *s: _rng.normal(s) * 0.05)(B, S, D)),
            "wqkv": _w((lambda *s: _rng.normal(s) * 0.05)(D, 3 * D)),
            "wo": _w((lambda *s: _rng.normal(s) * 0.05)(D, D)),
        }
    _A_in = _A_setup()

    def _B_setup():
        B, S, Dm, Df = 1, 2048, 1024, 3584
        return {
            "x": _w((lambda *s: _rng.normal(s) * 0.05)(B, S, Dm)),
            "w_gate": _w((lambda *s: _rng.normal(s) * 0.05)(Dm, Df) * (Dm ** -0.5)),
            "w_up": _w((lambda *s: _rng.normal(s) * 0.05)(Dm, Df) * (Dm ** -0.5)),
            "w_down": _w((lambda *s: _rng.normal(s) * 0.05)(Df, Dm) * (Df ** -0.5)),
        }
    _B_in = _B_setup()

    return {
        "A_x": _A_in["x"],
        "A_wqkv": _A_in["wqkv"],
        "A_wo": _A_in["wo"],
        "B_x": _B_in["x"],
        "B_w_gate": _B_in["w_gate"],
        "B_w_up": _B_in["w_up"],
        "B_w_down": _B_in["w_down"],
    }

def reference(A_x, A_wqkv, A_wo, B_x, B_w_gate, B_w_up, B_w_down):
    def _A_ref(x, wqkv, wo):
        B, S, D = x.shape
        H = 32; Dh = D // H
        W, dil = 8, 2
        qkv = (lambda x, *d: x.transpose(*d))((x @ wqkv).reshape(B, S, 3, H, Dh), 2, 0, 3, 1, 4)
        q, k, v = qkv[0], qkv[1], qkv[2]
        scale = Dh ** -0.5
        pos = jnp.arange(S)
        off = jnp.arange(W) * dil
        idx = pos[:, None] - off[None, :]
        mask = idx >= 0
        idx_c = jnp.where(mask, idx, 0).reshape(-1)
        kg = k[:, :, idx_c, :].reshape(B, H, S, W, Dh)
        vg = v[:, :, idx_c, :].reshape(B, H, S, W, Dh)
        logits = jnp.einsum("bhsd,bhswd->bhsw", q, kg) * scale
        logits = jnp.where(mask[None, None, :, :], logits, -1e9)
        attn = _softmax(logits, axis=-1)
        o = jnp.einsum("bhsw,bhswd->bhsd", attn, vg)
        return (lambda x, *d: x.transpose(*d))(o, 0, 2, 1, 3).reshape(B, S, D) @ wo

    def _B_ref(x, w_gate, w_up, w_down):
        g = jnp.einsum("bsd,df->bsf", x, w_gate)
        u = jnp.einsum("bsd,df->bsf", x, w_up)
        h = _gelu(g) * u
        return jnp.einsum("bsf,fd->bsd", h, w_down)

    x = A_x
    xn = _layernorm(x, axis=-1)
    return x + _A_ref(xn, A_wqkv, A_wo) + _B_ref(xn, B_w_gate, B_w_up, B_w_down)
```

```python
import functools
import jax
import jax.numpy as jnp
import numpy as np
from jax import lax
from jax.experimental import pallas as pl
from jax.experimental.pallas import tpu as pltpu

S, D, DF, H, DH, W, DIL = 2048, 1024, 3584, 32, 32, 8, 2
HALO = 16
L = 128
NG = D // L
HD = D // 2
KD = DF // 2
F32, BF16, U32 = jnp.float32, jnp.bfloat16, jnp.uint32
QUAD = ((0, 0), (0, 1), (1, 0), (1, 1))
XA, OA = 0, HD
P = functools.partial


def _dot(a, b):
    return jnp.dot(a, b, preferred_element_type=F32)


def _pk(x):
    return pltpu.bitcast(x.astype(BF16), U32)


def _un(x):
    return pltpu.bitcast(x, BF16)


def _ds(start, size, align=None):
    if not isinstance(start, int):
        start = pl.multiple_of(start, align or size)
    return pl.ds(start, size)


def _a_combos(a11, a12, a21, a22):
    return [a11 + a22, a21 + a22, a11, a22, a11 + a12, a21 - a11, a12 - a22]


def _b_combos(b11, b12, b21, b22):
    return [b11 + b22, b11, b12 - b22, b21 - b11, b22, b11 + b12, b21 + b22]


def _strassen(prod):
    m1 = prod(0)
    m2 = prod(1)
    c22 = m1 - m2
    m3 = prod(2)
    c22 = c22 + m3
    m4 = prod(3)
    c11 = m1 + m4
    c21 = m2 + m4
    m5 = prod(4)
    c11 = c11 - m5
    c12 = m3 + m5
    c22 = c22 + prod(5)
    c11 = c11 + prod(6)
    return c11, c12, c21, c22


class _Side:
    def __init__(self, nslots, lag, *jobs):
        self.at, self.gates, self.n = {}, {}, 0
        for fns, lo, hi, gate in jobs:
            hi = nslots - 1 + hi if hi <= 0 else hi
            for t, fn in enumerate(fns):
                k = lo + (t * (hi - lo + 1)) // len(fns)
                self.at.setdefault(k, []).append((fn, gate))
        self.lag = lag
        self.prev = []

    def tick(self, m):
        self.prev.append(m[:8, :L])
        todo = self.at.get(self.n, ())
        if self.lag is not None and self.n >= self.lag:
            for gate in dict.fromkeys(g for _, g in todo if g is not None):
                gate(self.prev[self.n - self.lag])
        for fn, _ in todo:
            fn()
        self.n += 1


def _split(n, parts):
    return [range(n * k // parts, n * (k + 1) // parts) for k in range(parts)]


def _perm_cols(blocks):
    rows = blocks[0].shape[0]
    lane = lax.broadcasted_iota(jnp.int32, (rows, L), 1)
    st = []
    for g in range(NG):
        t = ((lane >> 2) - g) & 31
        src = (lane & 3) * 32 + 4 * (t & 7) + (t >> 3)
        st.append(jnp.take_along_axis(blocks[g], src, axis=1))
    a = (lane >> 2) & 7
    cur = [st[(-j) % NG] for j in range(NG)]
    for b in (1, 2, 4):
        m = (a & b) != 0
        cur = [jnp.where(m, cur[(j - b) % NG], cur[j]) for j in range(NG)]
    return [cur[j] if j == 0 else pltpu.roll(cur[j], L - 4 * j, 1) for j in range(NG)]


def _gelu_mul(g, u):
    c0 = float(np.sqrt(2.0 / np.pi))
    th = jnp.tanh(g * (c0 + (c0 * 0.044715) * (g * g)))
    return ((0.5 * g) * u) * (1.0 + th)


def kernel(x_hbm, wqkv_hbm, wo_hbm, wg_hbm, wu_hbm, wd_hbm, o_ref,
           rqkv, ro, rg, ru, rd, wqkv_v, wgu_v, wdo_v, tmp_s, lhs_s, ha_s, qkv_s, x_s, sems,
           *, TM, FW, AG, AR, N1, N2, N3, LRC, ONLY, LAG, NPF):
    HM = TM // 2
    NC = KD // FW
    NGRP = HM // 16
    SCALE = DH ** -0.5
    i = pl.program_id(0)
    zero = i >> 16

    def cp_qkv(p):
        col = ((p + 1) % 3) * D
        return [pltpu.make_async_copy(wqkv_hbm.at[:, _ds(col, D)], rqkv.at[p], sems.at[p])]

    def cp_o():
        return [pltpu.make_async_copy(wo_hbm, ro, sems.at[3])]

    def cp_gu(c):
        return [pltpu.make_async_copy(w.at[:, _ds(nh * KD + c * FW, FW)], r.at[c, nh], sems.at[4 + c])
                for w, r in ((wg_hbm, rg), (wu_hbm, ru)) for nh in range(2)]

    def cp_d(c):
        return [pltpu.make_async_copy(wd_hbm.at[_ds(kh * KD + c * FW, FW), :], rd.at[c, kh], sems.at[4 + NC + c])
                for kh in range(2)]

    def cp_x(t):
        return [pltpu.make_async_copy(x_hbm.at[_ds(t * TM, TM), :], x_s.at[t % 2], sems.at[4 + 2 * NC])]

    def start(cps):
        for cp in cps:
            cp.start()

    def wait(cps):
        for cp in cps:
            cp.wait()

    def prep_gu(c, m, units):
        r = (rg, ru)[m]
        for u in units:
            t, n = divmod(u, FW // L)
            bs = [r[c, nh, kh * HD + t * 16:kh * HD + (t + 1) * 16, n * L:(n + 1) * L].astype(F32) for kh, nh in QUAD]
            col = (2 * n + m) * L
            for s, val in enumerate(_b_combos(*bs)):
                wgu_v.at[c + zero, s][t * 8:(t + 1) * 8, col:col + L] = _pk(val)

    def prep_d(c, units):
        for u in units:
            t, n = divmod(u, 4)
            bs = [rd[c, kh, t * 16:(t + 1) * 16, nh * HD + n * L:nh * HD + (n + 1) * L].astype(F32) for kh, nh in QUAD]
            for s, val in enumerate(_b_combos(*bs)):
                wdo_v.at[s][_ds(c * (FW // 2) + t * 8, 8), n * L:(n + 1) * L] = _pk(val)

    def prep_qkv(p, t, rc):
        half = []
        for kh in range(2):
            r = _ds(kh * HD + t * rc, rc)
            half.append(_perm_cols([pltpu.bitcast(rqkv[p, r, g * L:(g + 1) * L], U32) for g in range(NG)]))
        for n in range(4):
            bs = [_un(half[kh][nh * 4 + n]).astype(F32) for kh, nh in QUAD]
            for s, val in enumerate(_b_combos(*bs)):
                wqkv_v.at[p + zero, s][_ds(t * (rc // 2), rc // 2), n * L:(n + 1) * L] = _pk(val)

    def prep_o_stage(n, nh):
        g = nh * 4 + n
        for h in range(H):
            tmp_s[g, h * (DH + 1):h * (DH + 1) + DH, :] = ro[h * DH:(h + 1) * DH, g * L:(g + 1) * L].astype(F32)

    def prep_o(n, d0, nd):
        for d in range(d0, d0 + nd):
            bs = [tmp_s[nh * 4 + n, pl.ds(kh * (DH // 2) + d, H, stride=DH + 1), :] for kh, nh in QUAD]
            for s, val in enumerate(_b_combos(*bs)):
                wdo_v.at[s][KD // 2 + d * (H // 2):KD // 2 + (d + 1) * (H // 2), n * L:(n + 1) * L] = _pk(val)

    def layernorm(src_ref, t, rc):
        halves = []
        for base in (0, HM):
            x = src_ref[_ds(base + t * rc, rc), :].astype(F32)
            mu = jnp.mean(x, axis=-1, keepdims=True)
            xc = x - mu
            var = jnp.mean(xc * xc, axis=-1, keepdims=True)
            halves.append(xc * lax.rsqrt(var + 1e-5))
        a, b = halves
        for s, val in enumerate(_a_combos(a[:, :HD], a[:, HD:], b[:, :HD], b[:, HD:])):
            lhs_s.at[s + zero][_ds(t * (rc // 2), rc // 2), XA:XA + HD] = _pk(val)

    def attn_rows(r0, rc, dst):
        pos = i * TM + r0 + lax.broadcasted_iota(jnp.int32, (rc, L), 0)
        qs = [qkv_s[2, j, pl.ds(r0 + HALO, rc), :] for j in range(NG)]
        ss = []
        for w in range(W):
            s = None
            for j in range(NG):
                p = qs[j] * qkv_s[0, j, pl.ds(r0 + HALO - DIL * w, rc), :]
                s = p if s is None else s + p
            s = s + pltpu.roll(s, 64, 1)
            s = (s + pltpu.roll(s, 32, 1)) * SCALE
            if w > 0:
                s = jnp.where(pos >= DIL * w, s, -1e9)
            ss.append(s)
        m = functools.reduce(jnp.maximum, ss)
        ps = [jnp.exp(s - m) for s in ss]
        inv = 1.0 / functools.reduce(lambda a, b: a + b, ps)
        ps = [p * inv for p in ps]
        for j in range(NG):
            o = None
            for w in range(W):
                p = ps[w] * qkv_s[1, j, pl.ds(r0 + HALO - DIL * w, rc), :]
                o = p if o is None else o + p
            lhs_s.at[7 + zero][dst:dst + rc, j * L:(j + 1) * L] = pltpu.bitcast(o, U32)

    def attn_sums(grp):
        o = [pltpu.bitcast(lhs_s[7, rh * 16:(rh + 1) * 16, nh * HD:(nh + 1) * HD], F32) for rh, nh in QUAD]
        for s, val in enumerate(_a_combos(*o)):
            lhs_s.at[s + zero][_ds(grp * 8, 8), OA:OA + HD] = _pk(val)

    def attn_jobs(grp):
        out = []
        for rh in range(2):
            for t in range(16 // AR):
                r0 = grp * 16 + rh * HM + t * AR
                if not isinstance(r0, int):
                    r0 = pl.multiple_of(r0, AR)
                out.append(P(attn_rows, r0, AR, rh * 16 + t * AR))
        return out + [P(attn_sums, grp)]

    def gate_attn(v):
        qkv_s.at[2, zero][0:8, :] = v

    def gate_x(v):
        x_s.at[2 + zero].bitcast(U32)[0:8, 0:L] = pltpu.bitcast(v, U32)

    def gate_raw(ref):
        def gate(v):
            ref.at[ref.shape[0] - 1 + zero, 0][0:16, 0:L] = jnp.concatenate([v, v], axis=0).astype(BF16)
        return gate
    gate_g, gate_u, gate_d = gate_raw(rg), gate_raw(ru), gate_raw(rd)

    def qkv(p, *jobs):
        side = _Side(7 * (HD // N1), LAG, *jobs)
        for n0 in range(0, HD, N1):
            def prod(s):
                m = _dot(_un(lhs_s[s, :, XA:XA + HD]), _un(wqkv_v[p, s, :, n0:n0 + N1]))
                side.tick(m)
                return m
            for (rh, nh), cb in zip(QUAD, _strassen(prod)):
                for n in range(N1 // L):
                    qkv_s[p, nh * 4 + n0 // L + n, HALO + rh * HM:HALO + (rh + 1) * HM, :] = cb[:, n * L:(n + 1) * L]

    def gate_up(c, first):
        jobs = [(sum([attn_jobs(jnp.minimum(c * AG + a, NGRP - 1)) for a in range(AG)], []), 1, -1, gate_attn)]
        if first:
            @pl.when(c + 1 < NC)
            def _():
                wait(cp_gu(c + 1))
                start(cp_d(c + 1))

            @pl.when(c + 2 < NC)
            def _():
                start(cp_gu(c + 2))
            wait(cp_d(c))
            cn = jnp.minimum(c + 1, NC - 1)
            jobs.append(([P(prep_gu, cn, 0, u) for u in _split(32 * FW // L, NPF)], 1, -1, gate_g))
            jobs.append(([P(prep_gu, cn, 1, u) for u in _split(32 * FW // L, NPF)], 1, -1, gate_u))
            jobs.append(([P(prep_d, c, u) for u in _split(FW // 4, NPF)], 1, -1, gate_d))
        nsub = 2 * L // N2
        side = _Side(7 * (FW // L) * nsub, LAG, *jobs)
        for n in range(FW // L):
            def prod(s):
                ms = []
                for t in range(nsub):
                    col = 2 * L * n + t * N2
                    ms.append(_dot(_un(lhs_s[s, :, XA:XA + HD]), _un(wgu_v[c, s, :, col:col + N2])))
                    side.tick(ms[-1])
                return ms[0] if nsub == 1 else jnp.concatenate(ms, axis=1)
            hs = [_gelu_mul(cb[:, :L], cb[:, L:]) for cb in _strassen(prod)]
            for s, val in enumerate(_a_combos(*hs)):
                ha_s.at[s][:, _ds(c * FW + n * L, L)] = _pk(val)

    def down(t):
        nt = HD // N3
        per = HM // LRC // nt
        side = _Side(14, LAG, ([P(layernorm, x_s.at[(i + 1) % 2], t * per + r, LRC) for r in range(per)], 1, -1, gate_x))
        cols = _ds(t * N3, N3)
        KS = 1280

        def prod(s):
            m = None
            m = _dot(_un(ha_s[s, :, :KS]), _un(wdo_v[s, :KS // 2, cols]))
            side.tick(m)
            lhs = jnp.concatenate([_un(ha_s[s, :, KS:]), _un(lhs_s[s, :, OA:])], axis=1)
            d = _dot(lhs, _un(wdo_v[s, KS // 2:, cols]))
            side.tick(d)
            m = m + d
            return m
        for (rh, nh), cb in zip(QUAD, _strassen(prod)):
            rs = slice(rh * HM, (rh + 1) * HM)
            oc = _ds(nh * HD + t * N3, N3)
            o_ref[rs, oc] = (x_s[i % 2, rs, oc].astype(F32) + cb).astype(o_ref.dtype)

    if ONLY:
        if ONLY == "P2":
            pl.loop(0, NC)(lambda c: gate_up(c, False))
        if ONLY == "P2f":
            pl.loop(0, NC)(lambda c: gate_up(c, True))
        if ONLY == "P3":
            pl.loop(0, HD // N3)(down)
        if ONLY == "P1":
            pl.loop(0, 3)(qkv)
        if ONLY == "P1f":
            pl.loop(0, 2)(lambda p: qkv(p, ([P(prep_qkv, p + 1, t, 32) for t in range(16)], 0, -1, None)))
        return

    NT = S // TM

    @pl.when(jnp.logical_and(i > 0, i + 1 < NT))
    def _():
        start(cp_x(i + 1))

    @pl.when(i == 0)
    def _():
        start(cp_x(0))
        start(cp_qkv(0))
        wait(cp_x(0))
        pl.loop(0, HM // 32)(lambda t: layernorm(x_s.at[0], t, 32))
        wait(cp_qkv(0))
        start(cp_qkv(1))
        start(cp_qkv(2))
        pl.loop(0, HD // 64)(lambda t: prep_qkv(0, t, 64))

        @pl.loop(0, 2)
        def _(p):
            wait(cp_qkv(p + 1))
            start(cp_gu(p))

            @pl.when(p == 0)
            def _():
                start(cp_o())

            @pl.when(p == 1)
            def _():
                start(cp_d(0))
            qkv(p, ([P(prep_qkv, p + 1, t, 32) for t in range(16)], 0, -1, None))
        for j in range(NG):
            qkv_s[0, j, :HALO, :] = jnp.zeros((HALO, L), F32)
            qkv_s[1, j, :HALO, :] = jnp.broadcast_to(qkv_s[1, j, HALO:HALO + 1, :], (HALO, L))
        wait(cp_gu(0))
        wait(cp_o())
        start(cp_x(1))
        qkv(2, ([P(prep_gu, 0, m, u) for u in _split(32 * FW // L, 12) for m in range(2)], 0, -1, None),
            ([P(prep_o_stage, n, nh) for n in range(4) for nh in range(2)]
             + [P(prep_o, n, d0, 4) for n in range(4) for d0 in range(0, 16, 4)], 0, -1, None))
        pl.loop(0, NC)(lambda c: gate_up(c, True))

    @pl.when(i > 0)
    def _():
        pl.loop(0, 3)(qkv)
        pl.loop(0, NC)(lambda c: gate_up(c, False))

    for p in range(2):
        for j in range(NG):
            qkv_s[p, j, :HALO, :] = qkv_s[p, j, TM:, :]
    @pl.when(i + 1 < NT)
    def _():
        wait(cp_x(i + 1))
    if N3 == HD:
        down(0)
    else:
        pl.loop(0, HD // N3)(down)


def build(A_x, A_wqkv, A_wo, B_x, B_w_gate, B_w_up, B_w_down, TM=512, FW=256, AG=3, AR=8,
          N1=128, N2=128, N3=256, LRC=16, ONLY='', LAG=1, NPF=13):
    HM = TM // 2
    NC = KD // FW
    NT = S // TM
    x = A_x.reshape(S, D)
    any_spec = pl.BlockSpec(memory_space=pl.ANY)
    out = pl.pallas_call(
        P(kernel, TM=TM, FW=FW, AG=AG, AR=AR, N1=N1, N2=N2, N3=N3, LRC=LRC, ONLY=ONLY, LAG=LAG, NPF=NPF),
        grid=(NT,),
        in_specs=[any_spec] * 6,
        out_specs=pl.BlockSpec((TM, D), lambda i: (i, 0)),
        out_shape=jax.ShapeDtypeStruct((S, D), A_x.dtype),
        scratch_shapes=[
            pltpu.VMEM((3, D, D), BF16),
            pltpu.VMEM((D, D), BF16),
            pltpu.VMEM((NC + 1, 2, D, FW), BF16),
            pltpu.VMEM((NC + 1, 2, D, FW), BF16),
            pltpu.VMEM((NC + 1, 2, FW, D), BF16),
            pltpu.VMEM((3, 7, HD // 2, HD), U32),
            pltpu.VMEM((NC, 7, HD // 2, 2 * FW), U32),
            pltpu.VMEM((7, (KD + HD) // 2, HD), U32),
            pltpu.VMEM((NG, H * (DH + 1), L), F32),
            pltpu.VMEM((8, HM // 2, D), U32),
            pltpu.VMEM((7, HM // 2, KD), U32),
            pltpu.VMEM((3, NG, HALO + TM, L), F32),
            pltpu.VMEM((3, TM, D), BF16),
            pltpu.SemaphoreType.DMA((5 + 2 * NC,)),
        ],
        compiler_params=pltpu.CompilerParams(
            dimension_semantics=("arbitrary",), vmem_limit_bytes=124 * 1024 * 1024),
    )(x, A_wqkv, A_wo, B_w_gate, B_w_up, B_w_down)
    return out.reshape(A_x.shape)


@jax.jit
def pallas_parallel_sum__sliding_local_dilated__glu_gated_geglu__prompt_kernel(
        A_x, A_wqkv, A_wo, B_x, B_w_gate, B_w_up, B_w_down):
    return build(A_x, A_wqkv, A_wo, B_x, B_w_gate, B_w_up, B_w_down)
```

```python
import functools
import jax
import jax.numpy as jnp
import numpy as np
from jax import lax
from jax.experimental import pallas as pl
from jax.experimental.pallas import tpu as pltpu

S, D, DF, H, DH, W, DIL = 2048, 1024, 3584, 32, 32, 8, 2
L = 128
NG = D // L
HD, KD = D // 2, DF // 2
FW = 256
NC = KD // FW
NP = KD // L
TM = 512
HM = TM // 2
NGRP = HM // 16
HALO = 16
XA, OA = 0, HD
SCALE = DH ** -0.5
LOG2E = float(np.log2(np.e))
F32, BF16, U32 = jnp.float32, jnp.bfloat16, jnp.uint32
QUAD = ((0, 0), (0, 1), (1, 0), (1, 1))
P = functools.partial


def _dot(a, b):
    return jnp.dot(a, b, preferred_element_type=F32)


def _pk(x):
    return pltpu.bitcast(x.astype(BF16), U32)


def _un(x):
    return pltpu.bitcast(x, BF16)


def _ds(start, size, align=None):
    if not isinstance(start, int):
        start = pl.multiple_of(start, align or size)
    return pl.ds(start, size)


def _split(n, parts):
    return [range(n * k // parts, n * (k + 1) // parts) for k in range(parts)]


def _a_sums(a11, a12, a21, a22):
    return [a11 + a22, a21 + a22, a11, a22, a11 + a12, a21 - a11, a12 - a22]


def _b_sums(b11, b12, b21, b22):
    return [b11 + b22, b11, b12 - b22, b21 - b11, b22, b11 + b12, b21 + b22]


def _strassen(prod):
    m1 = prod(0)
    m2 = prod(1)
    c22 = m1 - m2
    m3 = prod(2)
    c22 = c22 + m3
    m4 = prod(3)
    c11 = m1 + m4
    c21 = m2 + m4
    m5 = prod(4)
    c11 = c11 - m5
    c12 = m3 + m5
    c22 = c22 + prod(5)
    c11 = c11 + prod(6)
    return c11, c12, c21, c22


def _now(x):
    return x


class _Side:
    def __init__(self, never, fence, jobs, lag=2):
        self.at, self.n, self.fence, self.lag, self.prev, self.never = {}, 0, fence, lag, [], never
        for pieces, lo, hi in jobs:
            lo = max(lo, lag)
            for t, piece in enumerate(pieces):
                self.at.setdefault(lo + (t * (hi - lo)) // len(pieces), []).append(piece)

    def tick(self, m):
        self.prev.append(m[:8, :L])
        todo = self.at.get(self.n, ())
        for fn in todo:
            fn(P(self.hold, self.prev[self.n - self.lag]))
        if todo:
            self.fence()
        self.n += 1

    def hold(self, v, x):
        if x.dtype != v.dtype:
            v = pltpu.bitcast(v, x.dtype)
        return jnp.where(self.never, jnp.tile(v, (x.shape[0] // 8, x.shape[1] // L)), x)


def _perm_cols(blocks):
    lane = lax.broadcasted_iota(jnp.int32, blocks[0].shape, 1)
    st = []
    for g in range(NG):
        t = ((lane >> 2) - g) & 31
        st.append(jnp.take_along_axis(blocks[g], (lane & 3) * 32 + 4 * (t & 7) + (t >> 3), axis=1))
    cur = [st[(-j) % NG] for j in range(NG)]
    for b in (1, 2, 4):
        m = ((lane >> 2) & b) != 0
        cur = [jnp.where(m, cur[(j - b) % NG], cur[j]) for j in range(NG)]
    return [cur[j] if j == 0 else pltpu.roll(cur[j], L - 4 * j, 1) for j in range(NG)]


def _gelu_mul(g, u):
    c0 = float(np.sqrt(2.0 / np.pi))
    th = jnp.tanh(g * (c0 + (c0 * 0.044715) * (g * g)))
    return ((0.5 * g) * u) * (1.0 + th)


def _kernel(x_hbm, wqkv_hbm, wo_hbm, wg_hbm, wu_hbm, wd_hbm, o_hbm,
            rqkv, rgu, rd, wqkv_v, wgu_v, wd_v, wo_v, tmp_s, lhs_s, ha_s, m_s, qkv_s, x_s, o_s,
            qsem, gsem, dsem, xsem, osem, *, PU, U1, U3, WPOS, QHI, ONLY):
    NT = x_hbm.shape[0] // TM
    i = pl.program_id(0)
    never = i < 0
    zero = i >> 16

    def cp_qkv(p):
        return [pltpu.make_async_copy(wqkv_hbm.at[:, pl.ds((p + 1) % 3 * D, D)], rqkv.at[p], qsem.at[p])]

    def cp_gu(c):
        return [pltpu.make_async_copy(w.at[:, _ds(nh * KD + c * FW, FW)], rgu.at[c, m, nh], gsem.at[c])
                for m, w in enumerate((wg_hbm, wu_hbm)) for nh in range(2)]

    def cp_o():
        return [pltpu.make_async_copy(wo_hbm.at[:, pl.ds((2 * a + b) * FW, FW)], rgu.at[NC, a, b], gsem.at[NC])
                for a, b in QUAD]

    def wait_gu(c):
        pltpu.make_async_copy(rgu.at[c], rgu.at[c], gsem.at[c]).wait()

    def cp_d(p):
        r0, n = (0, 608, 1200)[p], (608, 592, 592)[p]
        rows = [pl.ds(kh * KD + r0, n) for kh in range(2)]
        return [pltpu.make_async_copy(wd_hbm.at[r, :], rd.at[r, :], dsem.at[p]) for r in rows]

    def cp_x(t):
        return [pltpu.make_async_copy(x_hbm.at[_ds(t * TM, TM), :], x_s.at[t % 2], xsem)]

    def cp_out(t, n):
        cols = [pl.ds(nh * HD + n * L, L) for nh in range(2)]
        return [pltpu.make_async_copy(o_s.at[:, c], o_hbm.at[_ds(t * TM, TM), c], osem.at[n]) for c in cols]

    def start(cps):
        for cp in cps:
            cp.start()

    def wait(cps):
        for cp in cps:
            cp.wait()

    def held(b, hold):
        return _un(hold(pltpu.bitcast(b, U32)))

    def raw_sums(raw, hold):
        b11, b12, b21, b22 = raw
        return _b_sums(*[b.astype(F32) for b in (held(b11, hold), b12, b21, held(b22, hold))])

    def prep_gu(c, t0, units, hold=_now):
        for u in units:
            t, m, n = t0 + u // 4, u // 2 % 2, u % 2
            raw = [rgu[c, m, nh, _ds(kh * HD + t * 16, 16), pl.ds(n * L, L)] for kh, nh in QUAD]
            for s, val in enumerate(raw_sums(raw, hold)):
                wgu_v.at[2 * c + n, s][_ds(t * 8, 8), pl.ds(m * L, L)] = _pk(val)

    def prep_d(t0, units, hold):
        for u in units:
            t, n = t0 + u // 4, u % 4
            raw = [rd[_ds(kh * KD + t * 16, 16), pl.ds(nh * HD + n * L, L)] for kh, nh in QUAD]
            for s, val in enumerate(raw_sums(raw, hold)):
                wd_v.at[s][_ds(t * 8, 8), pl.ds(n * L, L)] = _pk(val)

    def prep_qkv(p, t, hold):
        half = []
        for kh in range(2):
            r = _ds(kh * HD + t * 32, 32)
            half.append(_perm_cols([hold(pltpu.bitcast(rqkv[p, r, pl.ds(g * L, L)], U32)) for g in range(NG)]))
        for n in range(4):
            for s, val in enumerate(_b_sums(*[_un(half[kh][nh * 4 + n]).astype(F32) for kh, nh in QUAD])):
                wqkv_v.at[p, s][_ds(t * 16, 16), pl.ds(n * L, L)] = _pk(val)

    def stage_o(n, slot, nh, hold):
        for h in range(H):
            raw = rgu[NC, nh, n // 2, pl.ds(h * DH, DH), _ds(n % 2 * L, L)]
            tmp_s[2 * slot + nh, pl.ds(h * (DH + 1), DH), :] = held(raw, hold).astype(F32)

    def prep_o(n, slot, ds, hold):
        for d in ds:
            bs = [hold(tmp_s[2 * slot + nh, pl.ds(kh * (DH // 2) + d, H, stride=DH + 1), :]) for kh, nh in QUAD]
            for s, val in enumerate(_b_sums(*bs)):
                wo_v.at[s][_ds(d * (H // 2), H // 2), _ds(n * L, L)] = _pk(val)

    def layernorm(src_ref, t, rc, hold=_now):
        halves = []
        for base in (0, HM):
            x = held(src_ref[_ds(base + t * rc, rc), :], hold).astype(F32)
            xc = x - jnp.mean(x, axis=-1, keepdims=True)
            var = jnp.mean(xc * xc, axis=-1, keepdims=True)
            halves.append(xc * lax.rsqrt(var + 1e-5))
        a, b = halves
        for s, val in enumerate(_a_sums(a[:, :HD], a[:, HD:], b[:, :HD], b[:, HD:])):
            lhs_s.at[s][_ds(t * (rc // 2), rc // 2), pl.ds(XA, HD)] = _pk(val)

    def attn_rows(r0, dst, masked, hold):
        qs = [hold(qkv_s[2, j, pl.ds(r0 + HALO, 8), :]) for j in range(NG)]
        ss = []
        for w in range(W):
            s = None
            for j in range(NG):
                p = qs[j] * qkv_s[0, j, pl.ds(r0 + HALO - DIL * w, 8), :]
                s = p if s is None else s + p
            s = s + pltpu.roll(s, 64, 1)
            s = s + pltpu.roll(s, 32, 1)
            if masked and w > 0:
                pos = i * TM + r0 + lax.broadcasted_iota(jnp.int32, (8, L), 0)
                s = jnp.where(pos >= DIL * w, s, -1e9 / SCALE)
            ss.append(s)
        m = functools.reduce(jnp.maximum, ss)
        ps = [jnp.exp2((s - m) * (SCALE * LOG2E)) for s in ss]
        inv = 1.0 / functools.reduce(lambda a, b: a + b, ps)
        ps = [p * inv for p in ps]
        for j in range(NG):
            o = None
            for w in range(W):
                p = ps[w] * qkv_s[1, j, pl.ds(r0 + HALO - DIL * w, 8), :]
                o = p if o is None else o + p
            lhs_s.at[7][pl.ds(dst, 8), pl.ds(j * L, L)] = pltpu.bitcast(o, U32)

    def attn_sums(grp, hold):
        o = [pltpu.bitcast(lhs_s[7, pl.ds(rh * 16, 16), pl.ds(nh * HD, HD)], F32) for rh, nh in QUAD]
        for s, val in enumerate(_a_sums(*o)):
            lhs_s.at[s][_ds(grp * 8, 8), pl.ds(OA, HD)] = _pk(val)

    def attn_pieces(grp, lead):
        out = []
        for rh, t in QUAD:
            r0 = grp * 16 + rh * HM + t * 8
            if not isinstance(r0, int):
                r0 = pl.multiple_of(r0, 8)
            out.append(P(attn_rows, r0, rh * 16 + t * 8, lead and rh == 0))
        return out + [P(attn_sums, grp)]

    def fence(dst, *srcs):
        for src in srcs:
            dst[0:8, 0:L] = src[0:8, 0:L]

    def xa(s):
        return _un(lhs_s[s, :, pl.ds(XA, HD)])

    def gate_up(c, npan, jobs=()):
        side = _Side(never, P(fence, wgu_v.at[NP + 1 + zero, 0], wqkv_v.at[zero, 0]), jobs)
        for n in range(npan):
            pan = c * npan + n

            def prod(s):
                ms = []
                for m in range(2):
                    ms.append(_dot(xa(s), _un(wgu_v[pan, s, :, pl.ds(m * L, L)])))
                    side.tick(ms[-1])
                return jnp.concatenate(ms, axis=1)
            hs = [_gelu_mul(cb[:, :L], cb[:, L:]) for cb in _strassen(prod)]
            for s, val in enumerate(_a_sums(*hs)):
                ha_s.at[s][:, _ds(pan * L, L)] = _pk(val)

    def qkv(p, jobs=()):
        side = _Side(never, P(fence, wqkv_v.at[3 + zero, 0], wd_v.at[zero], wo_v.at[zero]), jobs)
        for n in range(4):
            def prod(s):
                m = _dot(xa(s), _un(wqkv_v[p, s, :, pl.ds(n * L, L)]))
                side.tick(m)
                return m
            for (rh, nh), cb in zip(QUAD, _strassen(prod)):
                qkv_s[p, nh * 4 + n, pl.ds(HALO + rh * HM, HM), :] = cb

    def down(t):
        ng = NGRP // 2
        pieces = []
        for g in range(ng):
            pieces += attn_pieces(t * ng + g, g == 0)
            pieces.append(P(layernorm, x_s.at[(i + 1) % 2], t * ng + g, 16))
        side = _Side(never, P(fence, wd_v.at[7 + zero], lhs_s.at[zero]), [(pieces, 0, 7 * NC)])
        cols = _ds(t * 2 * L, 2 * L)
        for s in range(7):
            m = None
            for k in range(NC):
                d = _dot(_un(ha_s[s, :, pl.ds(k * FW, FW)]), _un(wd_v[s, pl.ds(k * FW // 2, FW // 2), cols]))
                side.tick(d)
                m = d if m is None else m + d
            m_s[s, :, cols] = m

    def out_proj():
        for n in range(4):
            cols = pl.ds(n * L, L)
            cs = _strassen(lambda s: m_s[s, :, cols] + _dot(_un(lhs_s[s, :, pl.ds(OA, HD)]), _un(wo_v[s, :, cols])))
            for (rh, nh), cb in zip(QUAD, cs):
                idx = (pl.ds(rh * HM, HM), pl.ds(nh * HD + n * L, L))
                o_s[idx] = (x_s[(i % 2,) + idx].astype(F32) + cb).astype(o_s.dtype)
            start(cp_out(i, n))

    def first_gate_up(c):
        for p in range(3):
            @pl.when(c == 2 * p + 1)
            def _():
                wait(cp_qkv(p))
                if p < 2:
                    start(cp_qkv(p + 1))

            @pl.when(c == 4 + p)
            def _():
                start(cp_d(p))

        def arrive(hold):
            wait_gu(c + 1)

            @pl.when(c + 2 < NC)
            def _():
                start(cp_gu(c + 2))

            @pl.when(c + 2 == NC)
            def _():
                start(cp_o())
        e = (c - 1) * 8
        p = jnp.where(c == 0, 3, e // 16)
        t0 = jnp.where(c == 0, 0, e % 16)
        gate_up(c, 2, [([P(prep_qkv, p, t0 + t) for t in range(8)], 0, QHI),
                       ([arrive], WPOS, WPOS + 1),
                       ([P(prep_gu, c + 1, 0, u) for u in _split(128, 27 - WPOS)], WPOS + 1, 28)])

    def first_qkv(p):
        for t in range(3):
            @pl.when(p == t)
            def _():
                wait(cp_d(t))
        pieces = [P(prep_d, 37 * p, u) for u in _split(38 * 4, 26)]
        opieces = [P(stage_o, p, 0, nh) for nh in range(2)] + [P(prep_o, p, 0, ds) for ds in _split(16, 8)]
        opieces += [P(stage_o, 3, 1, nh) for nh in range(2)]
        opieces += [P(prep_o, 3, 1, [5 * p + d for d in ds]) for ds in _split(6, 3)]
        qkv(p, [(pieces, 0, 28), (opieces, 0, 28)])

    def loop(n, fn, unroll):
        if unroll:
            for t in range(n):
                fn(t)
        else:
            pl.loop(0, n)(fn)

    if ONLY:
        if ONLY == "P2":
            pl.loop(0, NP // PU)(lambda c: gate_up(c, PU))
        if ONLY == "P2f":
            pl.loop(0, NC)(first_gate_up)
        if ONLY == "P1f":
            pl.loop(0, 3)(first_qkv)
        loop(2, down, U3)
        out_proj()
        for n in range(4):
            wait(cp_out(i, n))
        return

    @pl.when(i == 0)
    def _():
        start(cp_x(0))
        start(cp_gu(0))
        wait(cp_x(0))
        for t in range(HM // 32):
            layernorm(x_s.at[0], t, 32)
        wait_gu(0)
        start(cp_gu(1))
        start(cp_qkv(0))
        pl.loop(0, 4)(lambda t: prep_gu(0, t * 8, range(32)))
        pl.loop(0, NC)(first_gate_up)
        start(cp_x(1))
        pl.loop(0, 3)(first_qkv)
        for j in range(NG):
            qkv_s[0, j, :HALO, :] = jnp.zeros((HALO, L), F32)
            qkv_s[1, j, :HALO, :] = jnp.broadcast_to(qkv_s[1, j, HALO:HALO + 1, :], (HALO, L))

    @pl.when(i > 0)
    def _():
        @pl.when(i + 1 < NT)
        def _():
            start(cp_x(i + 1))
        pl.loop(0, NP // PU)(lambda c: gate_up(c, PU))
        loop(3, qkv, U1)

    @pl.when(i + 1 < NT)
    def _():
        wait(cp_x(i + 1))

    @pl.when(i > 0)
    def _():
        for n in range(4):
            wait(cp_out(i - 1, n))
    loop(2, down, U3)
    out_proj()
    for p in range(2):
        for j in range(NG):
            qkv_s[p, j, :HALO, :] = qkv_s[p, j, TM:, :]

    @pl.when(i == NT - 1)
    def _():
        for n in range(4):
            wait(cp_out(i, n))


def build(A_x, A_wqkv, A_wo, B_x, B_w_gate, B_w_up, B_w_down, PU=7, U1=0, U3=0, WPOS=10, QHI=28, ONLY=''):
    any_spec = pl.BlockSpec(memory_space=pl.ANY)
    out = pl.pallas_call(
        P(_kernel, PU=PU, U1=U1, U3=U3, WPOS=WPOS, QHI=QHI, ONLY=ONLY),
        grid=(S // TM,),
        in_specs=[any_spec] * 6,
        out_specs=any_spec,
        out_shape=jax.ShapeDtypeStruct((S, D), A_x.dtype),
        scratch_shapes=[
            pltpu.VMEM((4, D, D), BF16),
            pltpu.VMEM((NC + 1, 2, 2, D, FW), BF16),
            pltpu.VMEM((DF, D), BF16),
            pltpu.VMEM((4, 7, HD // 2, HD), U32),
            pltpu.VMEM((NP + 2, 7, HD // 2, 2 * L), U32),
            pltpu.VMEM((8, KD // 2, HD), U32),
            pltpu.VMEM((7, HD // 2, HD), U32),
            pltpu.VMEM((4, H * (DH + 1), L), F32),
            pltpu.VMEM((8, HM // 2, D), U32),
            pltpu.VMEM((7, HM // 2, KD), U32),
            pltpu.VMEM((7, HM, HD), F32),
            pltpu.VMEM((3, NG, HALO + TM, L), F32),
            pltpu.VMEM((2, TM, D), A_x.dtype),
            pltpu.VMEM((TM, D), A_x.dtype),
            pltpu.SemaphoreType.DMA((3,)),
            pltpu.SemaphoreType.DMA((NC + 1,)),
            pltpu.SemaphoreType.DMA((3,)),
            pltpu.SemaphoreType.DMA(()),
            pltpu.SemaphoreType.DMA((4,)),
        ],
        compiler_params=pltpu.CompilerParams(
            dimension_semantics=("arbitrary",), vmem_limit_bytes=124 * 1024 * 1024),
    )(A_x.reshape(S, D), A_wqkv, A_wo, B_w_gate, B_w_up, B_w_down)
    return out.reshape(A_x.shape)


@jax.jit
def pallas_parallel_sum__sliding_local_dilated__glu_gated_geglu__prompt_kernel(
        A_x, A_wqkv, A_wo, B_x, B_w_gate, B_w_up, B_w_down):
    return build(A_x, A_wqkv, A_wo, B_x, B_w_gate, B_w_up, B_w_down)
```

```python
import functools
import jax
import jax.numpy as jnp
import numpy as np
from jax import lax
from jax.experimental import pallas as pl
from jax.experimental.pallas import tpu as pltpu

S, D, DF, H, DH, W, DIL = 2048, 1024, 3584, 32, 32, 8, 2
L = 128
NG = D // L
HD, KD = D // 2, DF // 2
FW = 256
NC = KD // FW
NP = KD // L
TM = 512
HM = TM // 2
NGRP = HM // 16
HALO = 16
XA, OA = 0, HD
SCALE = DH ** -0.5
LOG2E = float(np.log2(np.e))
F32, BF16, U32 = jnp.float32, jnp.bfloat16, jnp.uint32
QUAD = ((0, 0), (0, 1), (1, 0), (1, 1))
P = functools.partial


def _dot(a, b):
    return jnp.dot(a, b, preferred_element_type=F32)


def _pk(x):
    return pltpu.bitcast(x.astype(BF16), U32)


def _un(x):
    return pltpu.bitcast(x, BF16)


def _ds(start, size, align=None):
    if not isinstance(start, int):
        start = pl.multiple_of(start, align or size)
    return pl.ds(start, size)


def _split(n, parts):
    return [range(n * k // parts, n * (k + 1) // parts) for k in range(parts)]


def _a_sums(a11, a12, a21, a22):
    return [a11 + a22, a21 + a22, a11, a22, a11 + a12, a21 - a11, a12 - a22]


def _b_sums(b11, b12, b21, b22):
    return [b11 + b22, b11, b12 - b22, b21 - b11, b22, b11 + b12, b21 + b22]


def _strassen(prod):
    m1 = prod(0)
    m2 = prod(1)
    c22 = m1 - m2
    m3 = prod(2)
    c22 = c22 + m3
    m4 = prod(3)
    c11 = m1 + m4
    c21 = m2 + m4
    m5 = prod(4)
    c11 = c11 - m5
    c12 = m3 + m5
    c22 = c22 + prod(5)
    c11 = c11 + prod(6)
    return c11, c12, c21, c22


def _now(x, *_):
    return x


class _Side:
    def __init__(self, never, fence, jobs, lag=2):
        self.at, self.n, self.fence, self.lag, self.prev, self.never = {}, 0, fence, lag, [], never
        for pieces, lo, hi in jobs:
            if not pieces:
                continue
            lo = max(lo, lag)
            for t, piece in enumerate(pieces):
                self.at.setdefault(lo + (t * (hi - lo)) // len(pieces), []).append(piece)

    def tick(self, m):
        self.prev.append(m)
        todo = self.at.get(self.n, ())
        for fn in todo:
            fn(P(self.hold, self.n))
        if todo:
            self.fence()
        self.n += 1

    def hold(self, n, x, frac=0.0, later=0):
        m = self.prev[n - self.lag + later]
        r = int(frac * (m.shape[0] // 8)) * 8
        v = m[r:r + 8, :L]
        if x.dtype != v.dtype:
            v = pltpu.bitcast(v, x.dtype)
        return jnp.where(self.never, jnp.tile(v, (x.shape[0] // 8, x.shape[1] // L)), x)


def _perm_cols(blocks):
    lane = lax.broadcasted_iota(jnp.int32, blocks[0].shape, 1)
    st = []
    for g in range(NG):
        t = ((lane >> 2) - g) & 31
        st.append(jnp.take_along_axis(blocks[g], (lane & 3) * 32 + 4 * (t & 7) + (t >> 3), axis=1))
    cur = [st[(-j) % NG] for j in range(NG)]
    for b in (1, 2, 4):
        m = ((lane >> 2) & b) != 0
        cur = [jnp.where(m, cur[(j - b) % NG], cur[j]) for j in range(NG)]
    return [cur[j] if j == 0 else pltpu.roll(cur[j], L - 4 * j, 1) for j in range(NG)]


def _gelu_mul(g, u):
    c0 = float(np.sqrt(2.0 / np.pi))
    th = jnp.tanh(g * (c0 + (c0 * 0.044715) * (g * g)))
    return ((0.5 * g) * u) * (1.0 + th)


def _kernel(x_hbm, wqkv_hbm, wo_hbm, wg_hbm, wu_hbm, wd_hbm, o_hbm,
            rqkv, rgu, rd, wqkv_v, wgu_v, wd_v, wo_v, tmp_s, lhs_s, ha_s, m_s, qkv_s, x_s, o_s,
            qsem, gsem, dsem, xsem, osem, *, PU, U1, U3, WPOS, QHI, ONLY, AV, ZIG, LAG3, NS, NX, STAG, FR, FQ, FL, FK):
    NT = x_hbm.shape[0] // TM
    i = pl.program_id(0)
    never = i < 0
    zero = i >> 16

    def cp_qkv(p):
        return [pltpu.make_async_copy(wqkv_hbm.at[:, pl.ds((p + 1) % 3 * D, D)], rqkv.at[p], qsem.at[p])]

    def cp_gu(c):
        return [pltpu.make_async_copy(w.at[:, _ds(c * 2 * FW, 2 * FW)], rgu.at[c, m], gsem.at[c])
                for m, w in enumerate((wg_hbm, wu_hbm))]

    def cp_o():
        return [pltpu.make_async_copy(wo_hbm.at[:, pl.ds(nh * HD, HD)], rgu.at[NC, nh], gsem.at[NC])
                for nh in range(2)]

    def wait_gu(c):
        pltpu.make_async_copy(rgu.at[c], rgu.at[c], gsem.at[c]).wait()

    def cp_d(p):
        r = pl.ds((0, 3, 5)[p] * 2 * FW, (3, 2, 2)[p] * 2 * FW)
        return [pltpu.make_async_copy(wd_hbm.at[r, :], rd.at[r, :], dsem.at[p])]

    def cp_x(t):
        rc = TM // NX
        return [pltpu.make_async_copy(x_hbm.at[_ds(t * TM + u * rc, rc), :], x_s.at[t % 2, pl.ds(u * rc, rc), :], xsem)
                for u in range(NX)]

    def cp_out(t, n):
        cols = [pl.ds(nh * HD + n * L, L) for nh in range(2)]
        return [pltpu.make_async_copy(o_s.at[:, c], o_hbm.at[_ds(t * TM, TM), c], osem.at[n]) for c in cols]

    def start(cps):
        for cp in cps:
            cp.start()

    def wait(cps):
        for cp in cps:
            cp.wait()

    def held(b, hold, frac=0.0):
        return _un(hold(pltpu.bitcast(b, U32), frac))

    def raw_sums(raw, hold, frac):
        b11, b12, b21, b22 = raw
        if not STAG & 1:
            frac = 0.0
        return _b_sums(*[b.astype(F32) for b in (held(b11, hold, frac), b12, b21, held(b22, hold, frac))])

    def prep_gu(c, t0, units, hold=_now):
        for k, u in enumerate(units):
            t, m, n = t0 + u // 4, u // 2 % 2, u % 2
            raw = [rgu[c, m, _ds(kh * HD + t * 16, 16), pl.ds(nh * FW + n * L, L)] for kh, nh in QUAD]
            for s, val in enumerate(raw_sums(raw, hold, k / len(units))):
                wgu_v.at[2 * c + n, s][_ds(t * 8, 8), pl.ds(m * L, L)] = _pk(val)

    def prep_d(t0, units, hold):
        for k, u in enumerate(units):
            t, n = t0 + u // 4, u % 4
            r0 = (t >> 4) * 2 * FW + (t & 15) * 16
            raw = [rd[_ds(r0 + kh * FW, 16), pl.ds(nh * HD + n * L, L)] for kh, nh in QUAD]
            for s, val in enumerate(raw_sums(raw, hold, k / len(units))):
                wd_v.at[s][_ds(t * 8, 8), pl.ds(n * L, L)] = _pk(val)

    def prep_qkv(p, t, hold):
        half = []
        for kh in range(2):
            r = _ds(kh * HD + t * 32, 32)
            half.append(_perm_cols([hold(pltpu.bitcast(rqkv[p, r, pl.ds(g * L, L)], U32), (kh * NG + g) / 16 * FQ)
                                    for g in range(NG)]))
        for n in range(4):
            for s, val in enumerate(_b_sums(*[_un(half[kh][nh * 4 + n]).astype(F32) for kh, nh in QUAD])):
                wqkv_v.at[p, s][_ds(t * 16, 16), pl.ds(n * L, L)] = _pk(val)

    def stage_o(n, slot, nh, hold):
        for h in range(H):
            raw = rgu[NC, nh, pl.ds(h * DH, DH), _ds(n * L, L)]
            tmp_s[2 * slot + nh, pl.ds(h * (DH + 1), DH), :] = held(raw, hold, h / H if STAG & 8 else 0.0).astype(F32)

    def prep_o(n, slot, ds, hold):
        for k, d in enumerate(ds):
            bs = [hold(tmp_s[2 * slot + nh, pl.ds(kh * (DH // 2) + d, H, stride=DH + 1), :], k / len(ds) if STAG & 8 else 0.0)
                  if kh == nh else tmp_s[2 * slot + nh, pl.ds(kh * (DH // 2) + d, H, stride=DH + 1), :] for kh, nh in QUAD]
            for s, val in enumerate(_b_sums(*bs)):
                wo_v.at[s][_ds(d * (H // 2), H // 2), _ds(n * L, L)] = _pk(val)

    def layernorm(src_ref, t, rc, hold=_now):
        halves = []
        for base in (0, HM):
            x = held(src_ref[_ds(base + t * rc, rc), :], hold, base / TM * FL).astype(F32)
            xc = x - jnp.mean(x, axis=-1, keepdims=True)
            var = jnp.mean(xc * xc, axis=-1, keepdims=True)
            halves.append(xc * lax.rsqrt(var + 1e-5))
        a, b = halves
        for s, val in enumerate(_a_sums(a[:, :HD], a[:, HD:], b[:, :HD], b[:, HD:])):
            lhs_s.at[s][_ds(t * (rc // 2), rc // 2), pl.ds(XA, HD)] = _pk(val)

    def attn_rows(r0, dst, masked, hold):
        def kv(p, j, w):
            return qkv_s[p, j, pl.ds(r0 + HALO - DIL * w, 8), :]
        if AV & 1:
            ss = [None] * W
            for j in range(NG):
                q = hold(kv(2, j, 0), j / NG * FK)
                for w in range(W):
                    p = q * kv(0, j, w)
                    ss[w] = p if j == 0 else ss[w] + p
        else:
            qs = [hold(kv(2, j, 0)) for j in range(NG)]
            ss = []
            for w in range(W):
                pr = [qs[j] * kv(0, j, w) for j in range(NG)]
                if AV & 2:
                    ss.append(((pr[0] + pr[1]) + (pr[2] + pr[3])) + ((pr[4] + pr[5]) + (pr[6] + pr[7])))
                else:
                    ss.append(functools.reduce(lambda a, b: a + b, pr))
        for w in range(W):
            s = ss[w]
            s = s + pltpu.roll(s, 64, 1)
            s = s + pltpu.roll(s, 32, 1)
            if masked and w > 0:
                pos = i * TM + r0 + lax.broadcasted_iota(jnp.int32, (8, L), 0)
                s = jnp.where(pos >= DIL * w, s, -1e9 / SCALE)
            ss[w] = s
        m = functools.reduce(jnp.maximum, ss)
        ps = [jnp.exp2((s - m) * (SCALE * LOG2E)) for s in ss]
        inv = 1.0 / functools.reduce(lambda a, b: a + b, ps)
        ps = [p * inv for p in ps]
        if STAG & 4:
            os_ = [None] * NG
            for w in range(W):
                p = hold(ps[w], w / W * FR, 1)
                for j in range(NG):
                    t = p * kv(1, j, w)
                    os_[j] = t if w == 0 else os_[j] + t
        else:
            os_ = [functools.reduce(lambda a, b: a + b, [ps[w] * kv(1, j, w) for w in range(W)]) for j in range(NG)]
        for j in range(NG):
            lhs_s.at[7][pl.ds(dst, 8), pl.ds(j * L, L)] = pltpu.bitcast(os_[j], U32)

    def attn_sums(grp, hold):
        o = [pltpu.bitcast(lhs_s[7, pl.ds(rh * 16, 16), pl.ds(nh * HD, HD)], F32) for rh, nh in QUAD]
        for s, val in enumerate(_a_sums(*o)):
            lhs_s.at[s][_ds(grp * 8, 8), pl.ds(OA, HD)] = _pk(val)

    def attn_pieces(grp, lead):
        out = []
        for rh, t in QUAD:
            r0 = grp * 16 + rh * HM + t * 8
            if not isinstance(r0, int):
                r0 = pl.multiple_of(r0, 8)
            out.append(P(attn_rows, r0, rh * 16 + t * 8, lead and rh == 0))
        return out + [P(attn_sums, grp)]

    def fence(dst, *srcs):
        for src in srcs:
            dst[0:8, 0:L] = src[0:8, 0:L]

    def xa(s):
        return _un(lhs_s[s, :, pl.ds(XA, HD)])

    def gate_up(c, npan, jobs=()):
        side = _Side(never, P(fence, wgu_v.at[NP + 1 + zero, 0], wqkv_v.at[zero, 0]), jobs)
        for n in range(npan):
            pan = c * npan + n

            def prod(s):
                ms = []
                for m in range(2):
                    ms.append(_dot(xa(s), _un(wgu_v[pan, s, :, pl.ds(m * L, L)])))
                    side.tick(ms[-1])
                return jnp.concatenate(ms, axis=1)
            hs = [_gelu_mul(cb[:, :L], cb[:, L:]) for cb in _strassen(prod)]
            for s, val in enumerate(_a_sums(*hs)):
                ha_s.at[s][:, _ds(pan * L, L)] = _pk(val)

    def qkv(p, jobs=()):
        side = _Side(never, P(fence, wqkv_v.at[3 + zero, 0], wd_v.at[zero], wo_v.at[zero]), jobs)
        for n in range(4):
            def prod(s):
                m = _dot(xa(s), _un(wqkv_v[p, s, :, pl.ds(n * L, L)]))
                side.tick(m)
                return m
            for (rh, nh), cb in zip(QUAD, _strassen(prod)):
                qkv_s[p, nh * 4 + n, pl.ds(HALO + rh * HM, HM), :] = cb

    def down(t):
        ng = NGRP // 2
        pieces = []
        for g in range(ng):
            if not AV & 8:
                pieces += attn_pieces(t * ng + g, g == 0)
            if not AV & 16:
                pieces.append(P(layernorm, x_s.at[(i + 1) % 2], t * ng + g, 16))
        side = _Side(never, P(fence, wd_v.at[7 + zero], lhs_s.at[zero]), [(pieces, 0, 7 * NC)], lag=LAG3)
        cols = _ds(t * 2 * L, 2 * L)

        def part(s, k0, k1, c0, nc):
            d = _dot(_un(ha_s[s, :, pl.ds(k0, k1 - k0)]),
                     _un(wd_v[s, pl.ds(k0 // 2, (k1 - k0) // 2), _ds(t * 2 * L + c0, nc, L)]))
            side.tick(d)
            return d
        for s in range(7):
            if ZIG:
                m = part(s, 0, 512, 0, L) + part(s, 512, 1024, 0, L) + part(s, 1024, 1536, 0, L)
                d = part(s, 1536, KD, 0, 2 * L)
                m_s[s, :, _ds(t * 2 * L, L)] = m + d[:, :L]
                m = d[:, L:] + part(s, 0, 512, L, L) + part(s, 512, 1024, L, L) + part(s, 1024, 1536, L, L)
                m_s[s, :, _ds(t * 2 * L + L, L)] = m
                continue
            m = None
            for k in range(NC):
                d = part(s, k * FW, (k + 1) * FW, 0, 2 * L)
                m = d if m is None else m + d
            m_s[s, :, cols] = m

    def out_proj():
        for n in range(4):
            cols = pl.ds(n * L, L)
            cs = _strassen(lambda s: m_s[s, :, cols] + _dot(_un(lhs_s[s, :, pl.ds(OA, HD)]), _un(wo_v[s, :, cols])))
            for (rh, nh), cb in zip(QUAD, cs):
                idx = (pl.ds(rh * HM, HM), pl.ds(nh * HD + n * L, L))
                o_s[idx] = (x_s[(i % 2,) + idx].astype(F32) + cb).astype(o_s.dtype)
            start(cp_out(i, n))

    def prep_chunk(c):
        pl.loop(0, 4)(lambda t: prep_gu(c, t * 8, range(32)))

    def first_gate_up(c):
        @pl.when(c > 0)
        def _():
            wait_gu(c + 1)

        @pl.when(c == 1)
        def _():
            wait_gu(1)
            prep_chunk(1)

        @pl.when(c + 2 < NC)
        def _():
            start(cp_gu(c + 2))

        @pl.when(c + 2 == NC)
        def _():
            start(cp_o())
        for p, (go, due) in enumerate(((0, 2), (1, 3), (3, 5))):
            @pl.when(c == go)
            def _():
                start(cp_qkv(p))

            @pl.when(c == due)
            def _():
                wait(cp_qkv(p))

            @pl.when(c == 4 + p)
            def _():
                start(cp_d(p))
        qp = []
        for j in range(10):
            e = (c - 2) * 10 + j
            ok = jnp.logical_and(e >= 0, e < 48)
            qp.append(P(prep_qkv, jnp.where(ok, e >> 4, 3), jnp.where(ok, e & 15, 0)))
        nxt = jnp.where(c == 0, NC, c + 1)
        gate_up(c, 2, [(qp, 0, QHI), ([P(prep_gu, nxt, 0, u) for u in _split(128, WPOS)], 0, 28)])

    def first_qkv(p):
        for t in range(3):
            @pl.when(p == t)
            def _():
                wait(cp_d(t))
        pieces = [P(prep_d, 37 * p, u) for u in _split(38 * 4, 26)]
        opieces = [P(stage_o, p, 0, nh) for nh in range(2)] + [P(prep_o, p, 0, ds) for ds in _split(16, 8)]
        opieces += [P(stage_o, 3, 1, nh) for nh in range(2)]
        opieces += [P(prep_o, 3, 1, [5 * p + d for d in ds]) for ds in _split(6, 3)]
        qkv(p, [(pieces, 0, 28), (opieces, 0, 28)])

    def loop(n, fn, unroll):
        if unroll:
            for t in range(n):
                fn(t)
        else:
            pl.loop(0, n)(fn)

    if ONLY:
        if ONLY == "P2":
            pl.loop(0, NP // PU)(lambda c: gate_up(c, PU))
        if ONLY == "P2f":
            pl.loop(0, NC)(first_gate_up)
        if ONLY == "P1f":
            pl.loop(0, 3)(first_qkv)
        loop(2, down, U3)
        out_proj()
        for n in range(4):
            wait(cp_out(i, n))
        return

    @pl.when(i == 0)
    def _():
        start(cp_x(0))
        start(cp_gu(0))
        wait(cp_x(0))
        for t in range(HM // 32):
            layernorm(x_s.at[0], t, 32)
        wait_gu(0)
        start(cp_gu(1))
        prep_chunk(0)
        pl.loop(0, NC)(first_gate_up)
        start(cp_x(1))
        pl.loop(0, 3)(first_qkv)
        for j in range(NG):
            qkv_s[0, j, :HALO, :] = jnp.zeros((HALO, L), F32)
            qkv_s[1, j, :HALO, :] = jnp.broadcast_to(qkv_s[1, j, HALO:HALO + 1, :], (HALO, L))

    @pl.when(i > 0)
    def _():
        @pl.when(i + 1 < NT)
        def _():
            start(cp_x(i + 1))
        pl.loop(0, NP // PU)(lambda c: gate_up(c, PU))
        loop(3, qkv, U1)

    @pl.when(i + 1 < NT)
    def _():
        wait(cp_x(i + 1))

    @pl.when(i > 0)
    def _():
        for n in range(4):
            wait(cp_out(i - 1, n))
    loop(2, down, U3)
    out_proj()
    for p in range(2):
        for j in range(NG):
            qkv_s[p, j, :HALO, :] = qkv_s[p, j, TM:, :]

    @pl.when(i == NT - 1)
    def _():
        for n in range(4):
            wait(cp_out(i, n))


def build(A_x, A_wqkv, A_wo, B_x, B_w_gate, B_w_up, B_w_down, PU=7, U1=0, U3=0, WPOS=26, QHI=28, AV=1, ZIG=1, LAG3=2, NS=1, STAG=15, FR=0.5, FQ=0.0, FL=1.0, FK=0.5, NX=1, ONLY=''):
    any_spec = pl.BlockSpec(memory_space=pl.ANY)
    out = pl.pallas_call(
        P(_kernel, PU=PU, U1=U1, U3=U3, WPOS=WPOS, QHI=QHI, ONLY=ONLY, AV=AV, ZIG=ZIG, LAG3=LAG3, NS=NS, NX=NX, STAG=STAG, FR=FR, FQ=FQ, FL=FL, FK=FK),
        grid=(S // TM,),
        in_specs=[any_spec] * 6,
        out_specs=any_spec,
        out_shape=jax.ShapeDtypeStruct((S, D), A_x.dtype),
        scratch_shapes=[
            pltpu.VMEM((4, D, D), BF16),
            pltpu.VMEM((NC + 1, 2, D, 2 * FW), BF16),
            pltpu.VMEM((DF, D), BF16),
            pltpu.VMEM((4, 7, HD // 2, HD), U32),
            pltpu.VMEM((NP + 2, 7, HD // 2, 2 * L), U32),
            pltpu.VMEM((8, KD // 2, HD), U32),
            pltpu.VMEM((7, HD // 2, HD), U32),
            pltpu.VMEM((4, H * (DH + 1), L), F32),
            pltpu.VMEM((8, HM // 2, D), U32),
            pltpu.VMEM((7, HM // 2, KD), U32),
            pltpu.VMEM((7, HM, HD), F32),
            pltpu.VMEM((3, NG, HALO + TM, L), F32),
            pltpu.VMEM((2, TM, D), A_x.dtype),
            pltpu.VMEM((TM, D), A_x.dtype),
            pltpu.SemaphoreType.DMA((3,)),
            pltpu.SemaphoreType.DMA((NC + 1,)),
            pltpu.SemaphoreType.DMA((3,)),
            pltpu.SemaphoreType.DMA(()),
            pltpu.SemaphoreType.DMA((4,)),
        ],
        compiler_params=pltpu.CompilerParams(
            dimension_semantics=("arbitrary",), vmem_limit_bytes=124 * 1024 * 1024),
    )(A_x.reshape(S, D), A_wqkv, A_wo, B_w_gate, B_w_up, B_w_down)
    return out.reshape(A_x.shape)


@jax.jit
def pallas_parallel_sum__sliding_local_dilated__glu_gated_geglu__prompt_kernel(
        A_x, A_wqkv, A_wo, B_x, B_w_gate, B_w_up, B_w_down):
    return build(A_x, A_wqkv, A_wo, B_x, B_w_gate, B_w_up, B_w_down)
```

```python
import functools

import jax
import jax.numpy as jnp
import numpy as np
from jax import lax
from jax.experimental import pallas as pl
from jax.experimental.pallas import tpu as pltpu

S, D, DF, H, DH, W, DIL = 2048, 1024, 3584, 32, 32, 8, 2
L = 128
NG = D // L
HD, KD = D // 2, DF // 2
FW = 256
NC = KD // FW
NP = KD // L
TM = 512
HM = TM // 2
HALO = 16
XA, OA = 0, HD
SCALE = DH ** -0.5
LOG2E = float(np.log2(np.e))
F32, BF16, U32 = jnp.float32, jnp.bfloat16, jnp.uint32
QUAD = ((0, 0), (0, 1), (1, 0), (1, 1))
P = functools.partial


def _dot(a, b):
    return jnp.dot(a, b, preferred_element_type=F32)


def _pack(x):
    return pltpu.bitcast(x.astype(BF16), U32)


def _unpack(x):
    return pltpu.bitcast(x, BF16)


def _ds(start, size, align=None):
    if not isinstance(start, int):
        start = pl.multiple_of(start, align or size)
    return pl.ds(start, size)


def _split(n, parts):
    return [range(n * k // parts, n * (k + 1) // parts) for k in range(parts)]


def _a_sums(a11, a12, a21, a22):
    return [a11 + a22, a21 + a22, a11, a22, a11 + a12, a21 - a11, a12 - a22]


def _b_sums(b11, b12, b21, b22):
    return [b11 + b22, b11, b12 - b22, b21 - b11, b22, b11 + b12, b21 + b22]


def _strassen(prod):
    m1 = prod(0)
    m2 = prod(1)
    c22 = m1 - m2
    m3 = prod(2)
    c22 = c22 + m3
    m4 = prod(3)
    c11 = m1 + m4
    c21 = m2 + m4
    m5 = prod(4)
    c11 = c11 - m5
    c12 = m3 + m5
    c22 = c22 + prod(5)
    c11 = c11 + prod(6)
    return c11, c12, c21, c22


def _now(x, *_):
    return x


class _Side:
    LAG = 2

    def __init__(self, never, fence, nslots, jobs):
        self.never, self.fence, self.at, self.prev = never, fence, {}, []
        for pieces in jobs:
            for t, piece in enumerate(pieces):
                self.at.setdefault(self.LAG + t * (nslots - self.LAG) // len(pieces), []).append(piece)

    def tick(self, m):
        n = len(self.prev)
        self.prev.append(m)
        for piece in self.at.get(n, ()):
            piece(P(self.hold, n - self.LAG))
        if n in self.at:
            self.fence()
        return m

    def hold(self, n, x, frac=0.0, later=0):
        m = self.prev[n + later]
        r = int(frac * (m.shape[0] // 8)) * 8
        v = m[r:r + 8, :L]
        if x.dtype != v.dtype:
            v = pltpu.bitcast(v, x.dtype)
        return jnp.where(self.never, jnp.tile(v, (x.shape[0] // 8, x.shape[1] // L)), x)


def _perm_cols(blocks):
    lane = lax.broadcasted_iota(jnp.int32, blocks[0].shape, 1)
    st = []
    for g in range(NG):
        t = ((lane >> 2) - g) & 31
        st.append(jnp.take_along_axis(blocks[g], (lane & 3) * 32 + 4 * (t & 7) + (t >> 3), axis=1))
    cur = [st[(-j) % NG] for j in range(NG)]
    for b in (1, 2, 4):
        m = ((lane >> 2) & b) != 0
        cur = [jnp.where(m, cur[(j - b) % NG], cur[j]) for j in range(NG)]
    return [cur[j] if j == 0 else pltpu.roll(cur[j], L - 4 * j, 1) for j in range(NG)]


def _gelu_mul(g, u):
    c0 = float(np.sqrt(2.0 / np.pi))
    th = jnp.tanh(g * (c0 + (c0 * 0.044715) * (g * g)))
    return ((0.5 * g) * u) * (1.0 + th)


def _kernel(x_hbm, wqkv_hbm, wo_hbm, wg_hbm, wu_hbm, wd_hbm, o_hbm,
            rqkv, rgu, rd, wqkv_v, wgu_v, wd_v, wo_v, tmp_s, lhs_s, ha_s, m_s, kvq_s, x_s, o_s,
            qsem, gsem, dsem, xsem, osem):
    nt = x_hbm.shape[0] // TM
    i = pl.program_id(0)
    never = i < 0
    zero = i >> 16

    def cp_qkv(p):
        return pltpu.make_async_copy(wqkv_hbm.at[:, pl.ds((p + 1) % 3 * D, D)], rqkv.at[p], qsem.at[p])

    def cp_gu(c, m):
        src = (wg_hbm, wu_hbm)[m].at[:, pl.ds(c * 2 * FW, 2 * FW)] if c < NC else wo_hbm.at[:, pl.ds(m * HD, HD)]
        return pltpu.make_async_copy(src, rgu.at[c, m], gsem.at[2 * c + m])

    def cp_d(p):
        rows = pl.ds((0, 3, 5)[p] * 2 * FW, (3, 2, 2)[p] * 2 * FW)
        return pltpu.make_async_copy(wd_hbm.at[rows, :], rd.at[rows, :], dsem.at[p])

    def cp_x(t):
        return pltpu.make_async_copy(x_hbm.at[_ds(t * TM, TM), :], x_s.at[t % 2], xsem)

    def cp_out(t, n, nh):
        cols = pl.ds(nh * HD + n * L, L)
        return pltpu.make_async_copy(o_s.at[:, cols], o_hbm.at[_ds(t * TM, TM), cols], osem.at[2 * n + nh])

    def held(b, hold, frac):
        return _unpack(hold(pltpu.bitcast(b, U32), frac))

    def raw_sums(raw, hold, frac):
        b11, b12, b21, b22 = raw
        return _b_sums(*[b.astype(F32) for b in (held(b11, hold, frac), b12, b21, held(b22, hold, frac))])

    def prep_gu(c, units, hold=_now):
        for k, (m, t, n) in enumerate(units):
            raw = [rgu[c, m, _ds(kh * HD + t * 16, 16), pl.ds(nh * FW + n * L, L)] for kh, nh in QUAD]
            for s, val in enumerate(raw_sums(raw, hold, k / len(units))):
                wgu_v.at[2 * c + n, s][_ds(t * 8, 8), pl.ds(m * L, L)] = _pack(val)

    def prep_gu_now(c, m):
        cp_gu(c, m).wait()
        pl.loop(0, 2)(lambda t: prep_gu(c, [(m, t * 16 + u, n) for u in range(16) for n in range(2)]))

    def prep_d(t0, units, hold):
        for k, u in enumerate(units):
            t, n = t0 + u // 4, u % 4
            r0 = (t >> 4) * 2 * FW + (t & 15) * 16
            raw = [rd[_ds(r0 + kh * FW, 16), pl.ds(nh * HD + n * L, L)] for kh, nh in QUAD]
            for s, val in enumerate(raw_sums(raw, hold, k / len(units))):
                wd_v.at[s][_ds(t * 8, 8), pl.ds(n * L, L)] = _pack(val)

    def prep_qkv(p, t, hold):
        rows = [_ds(kh * HD + t * 32, 32) for kh in range(2)]
        half = [_perm_cols([hold(pltpu.bitcast(rqkv[p, r, pl.ds(g * L, L)], U32)) for g in range(NG)]) for r in rows]
        for n in range(4):
            for s, val in enumerate(_b_sums(*[_unpack(half[kh][nh * 4 + n]).astype(F32) for kh, nh in QUAD])):
                wqkv_v.at[p, s][_ds(t * 16, 16), pl.ds(n * L, L)] = _pack(val)

    def stage_o(n, slot, nh, hold):
        for h in range(H):
            raw = rgu[NC, nh, pl.ds(h * DH, DH), _ds(n * L, L)]
            tmp_s[2 * slot + nh, pl.ds(h * (DH + 1), DH), :] = held(raw, hold, h / H).astype(F32)

    def prep_o(n, slot, ds, hold):
        for k, d in enumerate(ds):
            bs = [tmp_s[2 * slot + nh, pl.ds(kh * (DH // 2) + d, H, stride=DH + 1), :] for kh, nh in QUAD]
            bs[0], bs[3] = hold(bs[0], k / len(ds)), hold(bs[3], k / len(ds))
            for s, val in enumerate(_b_sums(*bs)):
                wo_v.at[s][_ds(d * (H // 2), H // 2), _ds(n * L, L)] = _pack(val)

    def layernorm(slot, t, rc, hold=_now):
        halves = []
        for rh in range(2):
            x = held(x_s[slot, _ds(rh * HM + t * rc, rc), :], hold, rh / 2).astype(F32)
            xc = x - jnp.mean(x, axis=-1, keepdims=True)
            var = jnp.mean(xc * xc, axis=-1, keepdims=True)
            halves.append(xc * lax.rsqrt(var + 1e-5))
        a, b = halves
        for s, val in enumerate(_a_sums(a[:, :HD], a[:, HD:], b[:, :HD], b[:, HD:])):
            lhs_s.at[s][_ds(t * (rc // 2), rc // 2), pl.ds(XA, HD)] = _pack(val)

    def attn_rows(r0, dst, masked, hold):
        def rows(p, j, w):
            return kvq_s[p, j, pl.ds(r0 + HALO - DIL * w, 8), :]
        ss = [None] * W
        for j in range(NG):
            q = hold(rows(2, j, 0), j / NG / 2)
            for w in range(W):
                t = q * rows(0, j, w)
                ss[w] = t if j == 0 else ss[w] + t
        for w in range(W):
            s = ss[w] + pltpu.roll(ss[w], 64, 1)
            s = s + pltpu.roll(s, 32, 1)
            if masked and w > 0:
                pos = i * TM + r0 + lax.broadcasted_iota(jnp.int32, (8, L), 0)
                s = jnp.where(pos >= DIL * w, s, -1e9 / SCALE)
            ss[w] = s
        m = functools.reduce(jnp.maximum, ss)
        es = [jnp.exp2((s - m) * (SCALE * LOG2E)) for s in ss]
        inv = 1.0 / functools.reduce(jnp.add, es)
        out = [None] * NG
        for w in range(W):
            p = hold(es[w] * inv, w / W, 1)
            for j in range(NG):
                t = p * rows(1, j, w)
                out[j] = t if w == 0 else out[j] + t
        for j in range(NG):
            lhs_s.at[7][pl.ds(dst, 8), pl.ds(j * L, L)] = pltpu.bitcast(out[j], U32)

    def attn_sums(grp, hold):
        o = [pltpu.bitcast(lhs_s[7, pl.ds(rh * 16, 16), pl.ds(nh * HD, HD)], F32) for rh, nh in QUAD]
        for s, val in enumerate(_a_sums(*o)):
            lhs_s.at[s][_ds(grp * 8, 8), pl.ds(OA, HD)] = _pack(val)

    def fence(dst, *srcs):
        for src in srcs:
            dst[0:8, 0:L] = src[0:8, 0:L]

    def xa(s):
        return _unpack(lhs_s[s, :, pl.ds(XA, HD)])

    def gate_up(c, npan, jobs=()):
        side = _Side(never, P(fence, wgu_v.at[NP + 1 + zero, 0], wqkv_v.at[zero, 0]), 14 * npan, jobs)
        for n in range(npan):
            pan = c * npan + n
            cs = _strassen(lambda s: jnp.concatenate(
                [side.tick(_dot(xa(s), _unpack(wgu_v[pan, s, :, pl.ds(m * L, L)]))) for m in range(2)], axis=1))
            for s, val in enumerate(_a_sums(*[_gelu_mul(cb[:, :L], cb[:, L:]) for cb in cs])):
                ha_s.at[s][:, _ds(pan * L, L)] = _pack(val)

    def qkv(p, jobs=()):
        side = _Side(never, P(fence, wqkv_v.at[3 + zero, 0], wd_v.at[zero], wo_v.at[zero]), 28, jobs)
        for n in range(4):
            cs = _strassen(lambda s: side.tick(_dot(xa(s), _unpack(wqkv_v[p, s, :, pl.ds(n * L, L)]))))
            for (rh, nh), cb in zip(QUAD, cs):
                kvq_s[p, nh * 4 + n, pl.ds(HALO + rh * HM, HM), :] = cb

    def down(t):
        pieces = []
        for g in range(8):
            grp = t * 8 + g
            for rh, u in QUAD:
                r0 = pl.multiple_of(grp * 16 + rh * HM + u * 8, 8)
                pieces.append(P(attn_rows, r0, rh * 16 + u * 8, g == 0 and rh == 0))
            pieces += [P(attn_sums, grp), P(layernorm, (i + 1) % 2, grp, 16)]
        side = _Side(never, P(fence, wd_v.at[7 + zero], lhs_s.at[zero]), 49, [pieces])

        def part(s, k0, k1, n, width=L):
            rhs = wd_v[s, pl.ds(k0 // 2, (k1 - k0) // 2), _ds((2 * t + n) * L, width, L)]
            return side.tick(_dot(_unpack(ha_s[s, :, pl.ds(k0, k1 - k0)]), _unpack(rhs)))
        for s in range(7):
            m = part(s, 0, 512, 0) + part(s, 512, 1024, 0) + part(s, 1024, 1536, 0)
            tail = part(s, 1536, KD, 0, 2 * L)
            m_s[s, :, _ds(2 * t * L, L)] = m + tail[:, :L]
            m = tail[:, L:] + part(s, 0, 512, 1) + part(s, 512, 1024, 1) + part(s, 1024, 1536, 1)
            m_s[s, :, _ds((2 * t + 1) * L, L)] = m

    def out_proj():
        for n in range(4):
            cols = pl.ds(n * L, L)
            cs = _strassen(lambda s: m_s[s, :, cols] + _dot(_unpack(lhs_s[s, :, pl.ds(OA, HD)]),
                                                            _unpack(wo_v[s, :, cols])))
            for (rh, nh), cb in zip(QUAD, cs):
                idx = (pl.ds(rh * HM, HM), pl.ds(nh * HD + n * L, L))
                o_s[idx] = (x_s[(i % 2,) + idx].astype(F32) + cb).astype(o_s.dtype)
            for nh in range(2):
                cp_out(i, n, nh).start()

    def first_gate_up(c):
        for cc in range(NC):
            @pl.when(c == cc)
            def _():
                for m in range(2):
                    if cc == 1:
                        prep_gu_now(1, m)
                    if cc > 0:
                        cp_gu(cc + 1, m).wait()
                    if cc + 2 <= NC:
                        cp_gu(cc + 2, m).start()
                for p, (go, due) in enumerate(((0, 2), (1, 3), (3, 5))):
                    if cc == go:
                        cp_qkv(p).start()
                    if cc == due:
                        cp_qkv(p).wait()
                if cc >= 4:
                    cp_d(cc - 4).start()
        qp = []
        for j in range(10):
            e = (c - 2) * 10 + j
            ok = jnp.logical_and(e >= 0, e < 48)
            qp.append(P(prep_qkv, jnp.where(ok, e >> 4, 3), jnp.where(ok, e & 15, 0)))
        nxt = jnp.where(c == 0, NC, c + 1)
        gate_up(c, 2, [qp, [P(prep_gu, nxt, [(u // 2 % 2, u // 4, u % 2) for u in us]) for us in _split(128, 26)]])

    def first_qkv(p):
        for t in range(3):
            pl.when(p == t)(cp_d(t).wait)
        dp = [P(prep_d, 37 * p, us) for us in _split(38 * 4, 26)]
        op = [P(stage_o, p, 0, nh) for nh in range(2)] + [P(prep_o, p, 0, ds) for ds in _split(16, 8)]
        op += [P(stage_o, 3, 1, nh) for nh in range(2)]
        op += [P(prep_o, 3, 1, [5 * p + d for d in ds]) for ds in _split(6, 3)]
        qkv(p, [dp, op])

    @pl.when(i == 0)
    def _():
        cp_x(0).start()
        cp_gu(0, 0).start()
        cp_x(0).wait()
        cp_gu(0, 1).start()
        pl.loop(0, 2)(lambda t: [layernorm(0, t * 4 + u, 32) for u in range(4)] and None)
        prep_gu_now(0, 0)
        cp_gu(1, 0).start()
        cp_gu(1, 1).start()
        prep_gu_now(0, 1)
        pl.loop(0, NC)(first_gate_up)
        cp_x(1).start()
        pl.loop(0, 3)(first_qkv)
        for j in range(NG):
            kvq_s[0, j, :HALO, :] = jnp.zeros((HALO, L), F32)
            kvq_s[1, j, :HALO, :] = jnp.broadcast_to(kvq_s[1, j, HALO:HALO + 1, :], (HALO, L))

    @pl.when(i > 0)
    def _():
        pl.when(i + 1 < nt)(cp_x(jnp.minimum(i + 1, nt - 1)).start)
        pl.loop(0, 2)(lambda c: gate_up(c, NP // 2))
        pl.loop(0, 3)(qkv)
        for n in range(4):
            for nh in range(2):
                cp_out(i - 1, n, nh).wait()

    pl.when(i + 1 < nt)(cp_x(jnp.minimum(i + 1, nt - 1)).wait)
    pl.loop(0, 2)(down)
    out_proj()
    for p in range(2):
        for j in range(NG):
            kvq_s[p, j, :HALO, :] = kvq_s[p, j, TM:, :]

    @pl.when(i == nt - 1)
    def _():
        for n in range(4):
            for nh in range(2):
                cp_out(i, n, nh).wait()


def build(A_x, A_wqkv, A_wo, B_x, B_w_gate, B_w_up, B_w_down, dummy=0):
    any_spec = pl.BlockSpec(memory_space=pl.ANY)
    out = pl.pallas_call(
        _kernel,
        grid=(S // TM,),
        in_specs=[any_spec] * 6,
        out_specs=any_spec,
        out_shape=jax.ShapeDtypeStruct((S, D), A_x.dtype),
        scratch_shapes=[
            pltpu.VMEM((4, D, D), BF16),
            pltpu.VMEM((NC + 1, 2, D, 2 * FW), BF16),
            pltpu.VMEM((DF, D), BF16),
            pltpu.VMEM((4, 7, HD // 2, HD), U32),
            pltpu.VMEM((NP + 2, 7, HD // 2, 2 * L), U32),
            pltpu.VMEM((8, KD // 2, HD), U32),
            pltpu.VMEM((7, HD // 2, HD), U32),
            pltpu.VMEM((4, H * (DH + 1), L), F32),
            pltpu.VMEM((8, HM // 2, D), U32),
            pltpu.VMEM((7, HM // 2, KD), U32),
            pltpu.VMEM((7, HM, HD), F32),
            pltpu.VMEM((3, NG, HALO + TM, L), F32),
            pltpu.VMEM((2, TM, D), A_x.dtype),
            pltpu.VMEM((TM, D), A_x.dtype),
            pltpu.SemaphoreType.DMA((3,)),
            pltpu.SemaphoreType.DMA((2 * NC + 2,)),
            pltpu.SemaphoreType.DMA((3,)),
            pltpu.SemaphoreType.DMA(()),
            pltpu.SemaphoreType.DMA((8,)),
        ],
        compiler_params=pltpu.CompilerParams(
            dimension_semantics=("arbitrary",), vmem_limit_bytes=124 * 1024 * 1024),
    )(A_x.reshape(S, D), A_wqkv, A_wo, B_w_gate, B_w_up, B_w_down)
    return out.reshape(A_x.shape)


@jax.jit
def pallas_parallel_sum__sliding_local_dilated__glu_gated_geglu__prompt_kernel(
        A_x, A_wqkv, A_wo, B_x, B_w_gate, B_w_up, B_w_down):
    return build(A_x, A_wqkv, A_wo, B_x, B_w_gate, B_w_up, B_w_down)
```

```python
import functools

import jax
import jax.numpy as jnp
import numpy as np
from jax import lax
from jax.experimental import pallas as pl
from jax.experimental.pallas import tpu as pltpu

S, D, DF, H, DH, W, DIL = 2048, 1024, 3584, 32, 32, 8, 2
L = 128
NG = D // L
HD, KD = D // 2, DF // 2
FW = 256
NC = KD // FW
NP = KD // L
TM = 512
HM = TM // 2
HALO = 16
XA, OA = 0, HD
SCALE = DH ** -0.5
LOG2E = float(np.log2(np.e))
F32, BF16, U32 = jnp.float32, jnp.bfloat16, jnp.uint32
QUAD = ((0, 0), (0, 1), (1, 0), (1, 1))
P = functools.partial


def _dot(a, b):
    return jnp.dot(a, b, preferred_element_type=F32)


def _pack(x):
    return pltpu.bitcast(x.astype(BF16), U32)


def _unpack(x):
    return pltpu.bitcast(x, BF16)


def _ds(start, size, align=None):
    if not isinstance(start, int):
        start = pl.multiple_of(start, align or size)
    return pl.ds(start, size)


def _split(n, parts):
    return [range(n * k // parts, n * (k + 1) // parts) for k in range(parts)]


def _a_sums(a11, a12, a21, a22):
    return [a11 + a22, a21 + a22, a11, a22, a11 + a12, a21 - a11, a12 - a22]


def _b_sums(b11, b12, b21, b22):
    return [b11 + b22, b11, b12 - b22, b21 - b11, b22, b11 + b12, b21 + b22]


def _strassen(prod):
    m1 = prod(0)
    m2 = prod(1)
    c22 = m1 - m2
    m3 = prod(2)
    c22 = c22 + m3
    m4 = prod(3)
    c11 = m1 + m4
    c21 = m2 + m4
    m5 = prod(4)
    c11 = c11 - m5
    c12 = m3 + m5
    c22 = c22 + prod(5)
    c11 = c11 + prod(6)
    return c11, c12, c21, c22


def _now(x, *_):
    return x


class _Side:
    LAG = 2

    def __init__(self, never, fence, nslots, jobs):
        self.never, self.fence, self.at, self.prev = never, fence, {}, []
        for pieces in jobs:
            for t, piece in enumerate(pieces):
                self.at.setdefault(self.LAG + t * (nslots - self.LAG) // len(pieces), []).append(piece)

    def tick(self, m):
        n = len(self.prev)
        self.prev.append(m)
        for piece in self.at.get(n, ()):
            piece(P(self.hold, n - self.LAG))
        if n in self.at:
            self.fence()
        return m

    def hold(self, n, x, frac=0.0, later=0):
        m = self.prev[n + later]
        r = int(frac * (m.shape[0] // 8)) * 8
        v = m[r:r + 8, :L]
        if x.dtype != v.dtype:
            v = pltpu.bitcast(v, x.dtype)
        return jnp.where(self.never, jnp.tile(v, (x.shape[0] // 8, x.shape[1] // L)), x)


def _perm_cols(blocks):
    lane = lax.broadcasted_iota(jnp.int32, blocks[0].shape, 1)
    st = []
    for g in range(NG):
        t = ((lane >> 2) - g) & 31
        st.append(jnp.take_along_axis(blocks[g], (lane & 3) * 32 + 4 * (t & 7) + (t >> 3), axis=1))
    cur = [st[(-j) % NG] for j in range(NG)]
    for b in (1, 2, 4):
        m = ((lane >> 2) & b) != 0
        cur = [jnp.where(m, cur[(j - b) % NG], cur[j]) for j in range(NG)]
    return [cur[j] if j == 0 else pltpu.roll(cur[j], L - 4 * j, 1) for j in range(NG)]


def _gelu_mul(g, u):
    c0 = float(np.sqrt(2.0 / np.pi))
    th = jnp.tanh(g * (c0 + (c0 * 0.044715) * (g * g)))
    return ((0.5 * g) * u) * (1.0 + th)


def _kernel(x_hbm, wqkv_hbm, wo_hbm, wg_hbm, wu_hbm, wd_hbm, o_hbm,
            rqkv, rgu, rd, wqkv_v, wgu_v, wd_v, wo_v, tmp_s, lhs_s, ha_s, m_s, kvq_s, x_s, o_s,
            qsem, gsem, dsem, xsem, osem):
    nt = x_hbm.shape[0] // TM
    i = pl.program_id(0)
    never = i < 0
    zero = i >> 16

    def cp_qkv(p):
        return pltpu.make_async_copy(wqkv_hbm.at[:, pl.ds((p + 1) % 3 * D, D)], rqkv.at[p], qsem.at[p])

    def cp_gu(c, m):
        src = (wg_hbm, wu_hbm)[m].at[:, pl.ds(c * 2 * FW, 2 * FW)] if c < NC else wo_hbm.at[:, pl.ds(m * HD, HD)]
        return pltpu.make_async_copy(src, rgu.at[c, m], gsem.at[2 * c + m])

    def cp_d(p):
        rows = pl.ds((0, 3, 5)[p] * 2 * FW, (3, 2, 2)[p] * 2 * FW)
        return pltpu.make_async_copy(wd_hbm.at[rows, :], rd.at[rows, :], dsem.at[p])

    def cp_x(t):
        return pltpu.make_async_copy(x_hbm.at[_ds(t * TM, TM), :], x_s.at[t % 2], xsem)

    def cp_out(t, n, nh):
        cols = pl.ds(nh * HD + n * L, L)
        return pltpu.make_async_copy(o_s.at[:, cols], o_hbm.at[_ds(t * TM, TM), cols], osem.at[2 * n + nh])

    def held(b, hold, frac):
        return _unpack(hold(pltpu.bitcast(b, U32), frac))

    def raw_sums(raw, hold, frac):
        b11, b12, b21, b22 = raw
        return _b_sums(*[b.astype(F32) for b in (held(b11, hold, frac), b12, b21, held(b22, hold, frac))])

    def prep_gu(c, units, hold=_now):
        for k, (m, t, n) in enumerate(units):
            raw = [rgu[c, m, _ds(kh * HD + t * 16, 16), pl.ds(nh * FW + n * L, L)] for kh, nh in QUAD]
            for s, val in enumerate(raw_sums(raw, hold, k / len(units))):
                wgu_v.at[2 * c + n, s][_ds(t * 8, 8), pl.ds(m * L, L)] = _pack(val)

    def prep_gu_now(c, m):
        cp_gu(c, m).wait()
        pl.loop(0, 2)(lambda t: prep_gu(c, [(m, t * 16 + u, n) for u in range(16) for n in range(2)]))

    def prep_d(t0, units, hold):
        for k, u in enumerate(units):
            t, n = t0 + u // 4, u % 4
            r0 = (t >> 4) * 2 * FW + (t & 15) * 16
            raw = [rd[_ds(r0 + kh * FW, 16), pl.ds(nh * HD + n * L, L)] for kh, nh in QUAD]
            for s, val in enumerate(raw_sums(raw, hold, k / len(units))):
                wd_v.at[s][_ds(t * 8, 8), pl.ds(n * L, L)] = _pack(val)

    def prep_qkv(p, t, hold):
        rows = [_ds(kh * HD + t * 32, 32) for kh in range(2)]
        half = [_perm_cols([hold(pltpu.bitcast(rqkv[p, r, pl.ds(g * L, L)], U32)) for g in range(NG)]) for r in rows]
        for n in range(4):
            for s, val in enumerate(_b_sums(*[_unpack(half[kh][nh * 4 + n]).astype(F32) for kh, nh in QUAD])):
                wqkv_v.at[p, s][_ds(t * 16, 16), pl.ds(n * L, L)] = _pack(val)

    def stage_o(n, slot, nh, hold):
        for h in range(H):
            raw = rgu[NC, nh, pl.ds(h * DH, DH), _ds(n * L, L)]
            tmp_s[2 * slot + nh, pl.ds(h * (DH + 1), DH), :] = held(raw, hold, h / H).astype(F32)

    def prep_o(n, slot, ds, hold):
        for k, d in enumerate(ds):
            bs = [tmp_s[2 * slot + nh, pl.ds(kh * (DH // 2) + d, H, stride=DH + 1), :] for kh, nh in QUAD]
            bs[0], bs[3] = hold(bs[0], k / len(ds)), hold(bs[3], k / len(ds))
            for s, val in enumerate(_b_sums(*bs)):
                wo_v.at[s][_ds(d * (H // 2), H // 2), _ds(n * L, L)] = _pack(val)

    def layernorm(slot, t, rc, hold=_now):
        halves = []
        for rh in range(2):
            x = held(x_s[slot, _ds(rh * HM + t * rc, rc), :], hold, rh / 2).astype(F32)
            xc = x - jnp.mean(x, axis=-1, keepdims=True)
            var = jnp.mean(xc * xc, axis=-1, keepdims=True)
            halves.append(xc * lax.rsqrt(var + 1e-5))
        a, b = halves
        for s, val in enumerate(_a_sums(a[:, :HD], a[:, HD:], b[:, :HD], b[:, HD:])):
            lhs_s.at[s][_ds(t * (rc // 2), rc // 2), pl.ds(XA, HD)] = _pack(val)

    def attn_rows(r0, dst, masked, hold):
        def rows(p, j, w):
            return kvq_s[p, j, pl.ds(r0 + HALO - DIL * w, 8), :]
        ss = [None] * W
        for j in range(NG):
            q = hold(rows(2, j, 0), j / NG / 2)
            for w in range(W):
                t = q * rows(0, j, w)
                ss[w] = t if j == 0 else ss[w] + t
        for w in range(W):
            s = ss[w] + pltpu.roll(ss[w], 64, 1)
            s = s + pltpu.roll(s, 32, 1)
            if masked and w > 0:
                pos = i * TM + r0 + lax.broadcasted_iota(jnp.int32, (8, L), 0)
                s = jnp.where(pos >= DIL * w, s, -1e9 / SCALE)
            ss[w] = s
        m = functools.reduce(jnp.maximum, ss)
        es = [jnp.exp2((s - m) * (SCALE * LOG2E)) for s in ss]
        inv = 1.0 / functools.reduce(jnp.add, es)
        out = [None] * NG
        for w in range(W):
            p = hold(es[w] * inv, w / W, 1)
            for j in range(NG):
                t = p * rows(1, j, w)
                out[j] = t if w == 0 else out[j] + t
        for j in range(NG):
            lhs_s.at[7][pl.ds(dst, 8), pl.ds(j * L, L)] = pltpu.bitcast(out[j], U32)

    def attn_sums(grp, hold):
        o = [pltpu.bitcast(lhs_s[7, pl.ds(rh * 16, 16), pl.ds(nh * HD, HD)], F32) for rh, nh in QUAD]
        for s, val in enumerate(_a_sums(*o)):
            lhs_s.at[s][_ds(grp * 8, 8), pl.ds(OA, HD)] = _pack(val)

    def fence(dst, *srcs):
        for src in srcs:
            dst[0:8, 0:L] = src[0:8, 0:L]

    def xa(s):
        return _unpack(lhs_s[s, :, pl.ds(XA, HD)])

    def gate_up(c, npan, jobs=()):
        side = _Side(never, P(fence, wgu_v.at[NP + 1 + zero, 0], wqkv_v.at[zero, 0]), 14 * npan, jobs)
        for n in range(npan):
            pan = c * npan + n
            cs = _strassen(lambda s: jnp.concatenate(
                [side.tick(_dot(xa(s), _unpack(wgu_v[pan, s, :, pl.ds(m * L, L)]))) for m in range(2)], axis=1))
            for s, val in enumerate(_a_sums(*[_gelu_mul(cb[:, :L], cb[:, L:]) for cb in cs])):
                ha_s.at[s][:, _ds(pan * L, L)] = _pack(val)

    def qkv(p, jobs=()):
        side = _Side(never, P(fence, wqkv_v.at[3 + zero, 0], wd_v.at[zero], wo_v.at[zero]), 28, jobs)
        for n in range(4):
            cs = _strassen(lambda s: side.tick(_dot(xa(s), _unpack(wqkv_v[p, s, :, pl.ds(n * L, L)]))))
            for (rh, nh), cb in zip(QUAD, cs):
                kvq_s[p, nh * 4 + n, pl.ds(HALO + rh * HM, HM), :] = cb

    def down(t):
        pieces = []
        for g in range(8):
            grp = t * 8 + g
            for rh, u in QUAD:
                r0 = pl.multiple_of(grp * 16 + rh * HM + u * 8, 8)
                pieces.append(P(attn_rows, r0, rh * 16 + u * 8, g == 0 and rh == 0))
            pieces += [P(attn_sums, grp), P(layernorm, (i + 1) % 2, grp, 16)]
        side = _Side(never, P(fence, wd_v.at[7 + zero], lhs_s.at[zero]), 49, [pieces])

        def part(s, k0, k1, n, width=L):
            rhs = wd_v[s, pl.ds(k0 // 2, (k1 - k0) // 2), _ds((2 * t + n) * L, width, L)]
            return side.tick(_dot(_unpack(ha_s[s, :, pl.ds(k0, k1 - k0)]), _unpack(rhs)))
        for s in range(7):
            m = part(s, 0, 512, 0) + part(s, 512, 1024, 0) + part(s, 1024, 1536, 0)
            tail = part(s, 1536, KD, 0, 2 * L)
            m_s[s, :, _ds(2 * t * L, L)] = m + tail[:, :L]
            m = tail[:, L:] + part(s, 0, 512, 1) + part(s, 512, 1024, 1) + part(s, 1024, 1536, 1)
            m_s[s, :, _ds((2 * t + 1) * L, L)] = m

    def out_proj():
        for n in range(4):
            cols = pl.ds(n * L, L)
            cs = _strassen(lambda s: m_s[s, :, cols] + _dot(_unpack(lhs_s[s, :, pl.ds(OA, HD)]),
                                                            _unpack(wo_v[s, :, cols])))
            for (rh, nh), cb in zip(QUAD, cs):
                idx = (pl.ds(rh * HM, HM), pl.ds(nh * HD + n * L, L))
                o_s[idx] = (x_s[(i % 2,) + idx].astype(F32) + cb).astype(o_s.dtype)
            for nh in range(2):
                cp_out(i, n, nh).start()

    def first_gate_up(c):
        for cc in range(NC):
            @pl.when(c == cc)
            def _():
                for m in range(2):
                    if cc == 1:
                        prep_gu_now(1, m)
                    if cc > 0:
                        cp_gu(cc + 1, m).wait()
                    if cc + 2 <= NC:
                        cp_gu(cc + 2, m).start()
                for p, (go, due) in enumerate(((0, 2), (1, 3), (3, 5))):
                    if cc == go:
                        cp_qkv(p).start()
                    if cc == due:
                        cp_qkv(p).wait()
                if cc >= 4:
                    cp_d(cc - 4).start()
        qp = []
        for j in range(10):
            e = (c - 2) * 10 + j
            ok = jnp.logical_and(e >= 0, e < 48)
            qp.append(P(prep_qkv, jnp.where(ok, e >> 4, 3), jnp.where(ok, e & 15, 0)))
        nxt = jnp.where(c == 0, NC, c + 1)
        gate_up(c, 2, [qp, [P(prep_gu, nxt, [(u // 2 % 2, u // 4, u % 2) for u in us]) for us in _split(128, 26)]])

    def first_qkv(p):
        for t in range(3):
            pl.when(p == t)(cp_d(t).wait)
        dp = [P(prep_d, 37 * p, us) for us in _split(38 * 4, 26)]
        op = [P(stage_o, p, 0, nh) for nh in range(2)] + [P(prep_o, p, 0, ds) for ds in _split(16, 8)]
        op += [P(stage_o, 3, 1, nh) for nh in range(2)]
        op += [P(prep_o, 3, 1, [5 * p + d for d in ds]) for ds in _split(6, 3)]
        qkv(p, [dp, op])

    @pl.when(i == 0)
    def _():
        cp_x(0).start()
        cp_gu(0, 0).start()
        cp_x(0).wait()
        cp_gu(0, 1).start()

        @pl.loop(0, 2)
        def _(t):
            for u in range(4):
                layernorm(0, t * 4 + u, 32)
        prep_gu_now(0, 0)
        cp_gu(1, 0).start()
        cp_gu(1, 1).start()
        prep_gu_now(0, 1)
        pl.loop(0, NC)(first_gate_up)
        cp_x(1).start()
        pl.loop(0, 3)(first_qkv)
        for j in range(NG):
            kvq_s[0, j, :HALO, :] = jnp.zeros((HALO, L), F32)
            kvq_s[1, j, :HALO, :] = jnp.broadcast_to(kvq_s[1, j, HALO:HALO + 1, :], (HALO, L))

    @pl.when(i > 0)
    def _():
        pl.when(i + 1 < nt)(cp_x(jnp.minimum(i + 1, nt - 1)).start)
        pl.loop(0, 2)(lambda c: gate_up(c, NP // 2))
        pl.loop(0, 3)(qkv)
        for n in range(4):
            for nh in range(2):
                cp_out(i - 1, n, nh).wait()

    pl.when(i + 1 < nt)(cp_x(jnp.minimum(i + 1, nt - 1)).wait)
    pl.loop(0, 2)(down)
    out_proj()
    for p in range(2):
        for j in range(NG):
            kvq_s[p, j, :HALO, :] = kvq_s[p, j, TM:, :]

    @pl.when(i == nt - 1)
    def _():
        for n in range(4):
            for nh in range(2):
                cp_out(i, n, nh).wait()


@jax.jit
def pallas_parallel_sum__sliding_local_dilated__glu_gated_geglu__prompt_kernel(
        A_x, A_wqkv, A_wo, B_x, B_w_gate, B_w_up, B_w_down):
    any_spec = pl.BlockSpec(memory_space=pl.ANY)
    out = pl.pallas_call(
        _kernel,
        grid=(S // TM,),
        in_specs=[any_spec] * 6,
        out_specs=any_spec,
        out_shape=jax.ShapeDtypeStruct((S, D), A_x.dtype),
        scratch_shapes=[
            pltpu.VMEM((4, D, D), BF16),
            pltpu.VMEM((NC + 1, 2, D, 2 * FW), BF16),
            pltpu.VMEM((DF, D), BF16),
            pltpu.VMEM((4, 7, HD // 2, HD), U32),
            pltpu.VMEM((NP + 2, 7, HD // 2, 2 * L), U32),
            pltpu.VMEM((8, KD // 2, HD), U32),
            pltpu.VMEM((7, HD // 2, HD), U32),
            pltpu.VMEM((4, H * (DH + 1), L), F32),
            pltpu.VMEM((8, HM // 2, D), U32),
            pltpu.VMEM((7, HM // 2, KD), U32),
            pltpu.VMEM((7, HM, HD), F32),
            pltpu.VMEM((3, NG, HALO + TM, L), F32),
            pltpu.VMEM((2, TM, D), A_x.dtype),
            pltpu.VMEM((TM, D), A_x.dtype),
            pltpu.SemaphoreType.DMA((3,)),
            pltpu.SemaphoreType.DMA((2 * NC + 2,)),
            pltpu.SemaphoreType.DMA((3,)),
            pltpu.SemaphoreType.DMA(()),
            pltpu.SemaphoreType.DMA((8,)),
        ],
        compiler_params=pltpu.CompilerParams(
            dimension_semantics=("arbitrary",), vmem_limit_bytes=120 * 1024 * 1024),
    )(A_x.reshape(S, D), A_wqkv, A_wo, B_w_gate, B_w_up, B_w_down)
    return out.reshape(A_x.shape)
```
